```python
import jax
import jax.numpy as jnp

def _softmax(x, axis=-1):
    return jax.nn.softmax(x, axis=axis)
def _gelu(x):
    return jax.nn.gelu(x, approximate=True)
def _silu(x):
    return jax.nn.silu(x)
def _sigmoid(x):
    return jax.nn.sigmoid(x)
def _layernorm(x, axis=-1, eps=1e-5):
    m = jnp.mean(x, axis=axis, keepdims=True)
    v = jnp.var(x, axis=axis, keepdims=True)
    return (x - m) / jnp.sqrt(v + eps)
def _scatter_add(tgt, idx, src, axis=0):
    return tgt.at[idx].add(src)
def _segment_sum(src, seg, n):
    return jax.ops.segment_sum(src, seg, n)
class _Rng:
    def __init__(self, key):
        self._k = key
    def _next(self):
        self._k, sub = jax.random.split(self._k)
        return sub
    def normal(self, shape):
        return jax.random.normal(self._next(), shape, dtype=jnp.bfloat16)
    def randint(self, lo, hi, shape):
        return jax.random.randint(self._next(), shape, lo, hi, dtype=jnp.int32)
    def uniform(self, shape, lo=0.0, hi=1.0):
        return jax.random.uniform(self._next(), shape, jnp.bfloat16, lo, hi)
    def permutation(self, n):
        return jax.random.permutation(self._next(), n)


kernel_name = 'gated_mix__compressed_kv_cla__sliding_block_cached__decode'

def setup_inputs():
    _rng = _Rng(jax.random.key(int.from_bytes(__import__("os").urandom(4), "little")))
    _w = (lambda a: (lambda t: t.astype(jnp.bfloat16) if jnp.issubdtype(t.dtype, jnp.floating) else t)(jnp.asarray(a)))
    def _A_setup():
        B, H, Sq, Sk, D, M = 8, 32, 1, 4096, 128, 512
        Dc = 4 * D
        return {
            "x": _w((lambda *s: _rng.normal(s) * 0.05)(B, Sq, M)),
            "c_kv": _w((lambda *s: _rng.normal(s) * 0.05)(B, Sk, Dc)),
            "w_q": _w((lambda *s: _rng.normal(s) * 0.05)(M, H, D) * (M ** -0.5)),
            "w_uk": _w((lambda *s: _rng.normal(s) * 0.05)(Dc, H, D) * (Dc ** -0.5)),
            "w_uv": _w((lambda *s: _rng.normal(s) * 0.05)(Dc, H, D) * (Dc ** -0.5)),
            "w_o": _w((lambda *s: _rng.normal(s) * 0.05)(H, D, M) * ((H * D) ** -0.5)),
        }
    _A_in = _A_setup()

    def _B_setup():
        B, Sq, D = 8, 1, 512
        Hq, Hkv, Sk, Dh = 32, 8, 4096, 128
        assert Hq % Hkv == 0, (Hq, Hkv)
        return {
            "x": _w((lambda *s: _rng.normal(s) * 0.05)(B, Sq, D)),
            "k_cache": _w((lambda *s: _rng.normal(s) * 0.05)(B, Hkv, Sk, Dh)),
            "v_cache": _w((lambda *s: _rng.normal(s) * 0.05)(B, Hkv, Sk, Dh)),
            "wq": _w((lambda *s: _rng.normal(s) * 0.05)(D, Hq * Dh) * (D ** -0.5)),
            "wo": _w((lambda *s: _rng.normal(s) * 0.05)(Hq * Dh, D) * ((Hq * Dh) ** -0.5)),
        }
    _B_in = _B_setup()

    return {
        "A_x": _A_in["x"],
        "A_c_kv": _A_in["c_kv"],
        "A_w_q": _A_in["w_q"],
        "A_w_uk": _A_in["w_uk"],
        "A_w_uv": _A_in["w_uv"],
        "A_w_o": _A_in["w_o"],
        "B_x": _B_in["x"],
        "B_k_cache": _B_in["k_cache"],
        "B_v_cache": _B_in["v_cache"],
        "B_wq": _B_in["wq"],
        "B_wo": _B_in["wo"],
        "gate_w": _w((lambda *s: _rng.normal(s) * 0.05)(512)),
    }

def reference(A_x, A_c_kv, A_w_q, A_w_uk, A_w_uv, A_w_o, B_x, B_k_cache, B_v_cache, B_wq, B_wo, gate_w):
    def _A_ref(x, c_kv, w_q, w_uk, w_uv, w_o):
        B, Sq, M = x.shape[0], x.shape[1], x.shape[2]
        Sk = c_kv.shape[1]
        H, D = w_q.shape[1], w_q.shape[2]
        q = jnp.einsum("bqm,mhd->bhqd", x, w_q)
        k = jnp.einsum("bkc,chd->bhkd", c_kv, w_uk)
        v = jnp.einsum("bkc,chd->bhkd", c_kv, w_uv)
        scores = jnp.einsum("bhqd,bhkd->bhqk", q, k) * (D ** -0.5)
        off = Sk - Sq
        qi = jnp.arange(Sq)[:, None]
        kj = jnp.arange(Sk)[None, :]
        cmask = kj <= (qi + off)
        scores = jnp.where(cmask[None, None], scores, -1e9)
        p = _softmax(scores, axis=-1)
        ctx = jnp.einsum("bhqk,bhkd->bhqd", p, v)
        return jnp.einsum("bhqd,hdm->bqm", ctx, w_o)

    def _B_ref(x, k_cache, v_cache, wq, wo):
        B, Sq, D = x.shape
        Hq, Dh = 32, 128
        Hkv, Sk = k_cache.shape[1], k_cache.shape[2]
        W = min(4096, max(256, Sk // 4))
        rep = Hq // Hkv
        q = (lambda x, *d: x.transpose(*d))((x @ wq).reshape(B, Sq, Hq, Dh), 0, 2, 1, 3)
        k = jnp.repeat(k_cache[:, :, Sk - W:, :], rep, axis=1)
        v = jnp.repeat(v_cache[:, :, Sk - W:, :], rep, axis=1)
        scores = jnp.einsum("bhqd,bhkd->bhqk", q, k) * (Dh ** -0.5)
        p = _softmax(scores, axis=-1)
        o = jnp.einsum("bhqk,bhkd->bhqd", p, v)
        return (lambda x, *d: x.transpose(*d))(o, 0, 2, 1, 3).reshape(B, Sq, Hq * Dh) @ wo

    x = A_x
    g = _sigmoid((x * gate_w).sum(-1, keepdims=True))
    a = _A_ref(x, A_c_kv, A_w_q, A_w_uk, A_w_uv, A_w_o)
    b = _B_ref(x, B_k_cache, B_v_cache, B_wq, B_wo)
    return g * a + (1 - g) * b
```

```python
import jax
import jax.numpy as jnp
from jax import lax
import jax.experimental.pallas as pl
import jax.experimental.pallas.tpu as pltpu

_BF = jnp.bfloat16
_F32 = jnp.float32
_NT = (((1,), (1,)), ((), ()))


def _dot(a, b):
    return jnp.dot(a, b, preferred_element_type=_F32)


def _dot_nt(a, b):
    return lax.dot_general(a, b, _NT, preferred_element_type=_F32)


def _head_pairs(w_ref, n_rows, n_heads, fn):
    w32 = w_ref.bitcast(jnp.uint32)
    npair = n_heads // 2
    grp = 4
    half = n_rows // 2
    span = n_rows * npair - (npair - grp)

    def body(jj, carry):
        sub = w32.at[pl.ds(pl.multiple_of(jj * grp, grp), span), :]
        for r in range(grp):
            ev = sub[pl.ds(r, half, stride=2 * npair), :]
            od = sub[pl.ds(r + npair, half, stride=2 * npair), :]
            lo = (ev & jnp.uint32(0xFFFF)) | (od << 16)
            hi = (ev >> 16) | (od & jnp.uint32(0xFFFF0000))
            h = 2 * (jj * grp + r)
            fn(h, pltpu.bitcast(lo, _BF))
            fn(h + 1, pltpu.bitcast(hi, _BF))
        return carry

    lax.fori_loop(0, npair // grp, body, 0)


@jax.jit
def pallas_gated_mix__compressed_kv_cla__sliding_block_cached__decode_kernel(
    A_x: jax.Array,
    A_c_kv: jax.Array,
    A_w_q: jax.Array,
    A_w_uk: jax.Array,
    A_w_uv: jax.Array,
    A_w_o: jax.Array,
    B_x: jax.Array,
    B_k_cache: jax.Array,
    B_v_cache: jax.Array,
    B_wq: jax.Array,
    B_wo: jax.Array,
    gate_w: jax.Array,
):
    del B_x
    B, Sq, M = A_x.shape
    Sk, Dc = A_c_kv.shape[1], A_c_kv.shape[2]
    H, D = A_w_q.shape[1], A_w_q.shape[2]
    Hq, Dh = 32, 128
    Hkv, SkB = B_k_cache.shape[1], B_k_cache.shape[2]
    W = min(4096, max(256, SkB // 4))
    rep = Hq // Hkv
    assert Sq == 1 and B == 8 and D == 128 and Dh == 128 and rep == 4 and H == Hq
    nck = Dc // 128
    scale_a = float(D) ** -0.5
    scale_b = float(Dh) ** -0.5
    wo_parts = ((0, 24), (24, 30), (30, 32))

    def kernel(x_hbm, c_hbm, wq_hbm, wuk_hbm, wuv_hbm, wo_hbm, k_hbm, v_hbm, bwq_hbm, bwo_hbm,
               gw_hbm, o_ref,
               x_s, gw_s, c_s, wq_s, wuk_s, wuv_s, wo_s, k_s, v_s, bwq_s, bwo_s,
               qb_s, qa_s, qabs_s, cabs_s, ctx_s, ob_s, sems):

        def cp(src, dst, s):
            return pltpu.make_async_copy(src, dst, sems.at[s])

        def c_copy(b, s):
            return cp(c_hbm.at[b], c_s.at[b], s)

        def kv_copies(b, s):
            return (cp(k_hbm.at[b, :, pl.ds(SkB - W, W), :], k_s.at[b], s),
                    cp(v_hbm.at[b, :, pl.ds(SkB - W, W), :], v_s.at[b], s))

        def bwo_copy(i, s):
            lo, hi = wo_parts[i]
            rows = pl.ds(lo * Dh, (hi - lo) * Dh)
            return cp(bwo_hbm.at[rows, :], bwo_s.at[rows, :], s)

        first = (cp(bwq_hbm, bwq_s, 0), cp(x_hbm, x_s, 0), cp(gw_hbm, gw_s, 0))
        for d in first:
            d.start()
        cp(wq_hbm, wq_s, 1).start()
        cp(wuk_hbm, wuk_s, 2).start()
        c_copy(0, 3).start()

        for d in first:
            d.wait()
        for d in kv_copies(0, 0):
            d.start()
        x = x_s[...].reshape(B, M)
        xf = x.astype(_F32)
        gate = jax.nn.sigmoid(
            jnp.sum(xf * gw_s[...].reshape(1, M).astype(_F32), axis=-1, keepdims=True))

        def qb_body(g, carry):
            cols = pl.ds(pl.multiple_of(g * (8 * Dh), 8 * Dh), 8 * Dh)
            q = _dot(x, bwq_s[:, cols]).astype(_BF).astype(_F32) * scale_b
            for r in range(8):
                row = pl.multiple_of((g * 8 + r) * B, B)
                qb_s[pl.ds(row, B), :] = q[:, r * Dh:(r + 1) * Dh]
            return carry

        lax.fori_loop(0, Hq // 8, qb_body, 0)

        cp(wq_hbm, wq_s, 1).wait()
        c_copy(1, 1).start()

        def qa_fn(h, w):
            qa_s[pl.ds(pl.multiple_of(h * B, B), B), :] = _dot(x, w)

        _head_pairs(wq_s, M, H, qa_fn)

        cp(wuk_hbm, wuk_s, 2).wait()
        for d in kv_copies(1, 2):
            d.start()

        def qabs_fn(h, w):
            rows = pl.ds(pl.multiple_of(h * B, B), B)
            r = _dot_nt(qa_s[rows, :].astype(_BF), w) * scale_a
            for k in range(nck):
                qabs_s[k, rows, :] = r[:, k * 128:(k + 1) * 128]

        _head_pairs(wuk_s, Dc, H, qabs_fn)

        def batch_body(b, carry):
            sc = jnp.where(b % 2 == 0, 3, 1)
            sk = jnp.where(b % 2 == 0, 0, 2)

            c_copy(b, sc).wait()

            @pl.when(b + 2 < B)
            def _():
                c_copy(b + 2, sc).start()

            @pl.when(b == B - 2)
            def _():
                cp(wuv_hbm, wuv_s, sc).start()

            @pl.when(b == B - 1)
            def _():
                bwo_copy(0, sc).start()

            q = jnp.concatenate([qabs_s[k, pl.ds(b, H, stride=B), :] for k in range(nck)],
                                axis=1).astype(_BF)
            c = c_s[b]
            s = _dot_nt(q, c)
            m = jnp.max(s, axis=-1, keepdims=True)
            p = jnp.exp(s - m)
            l = jnp.sum(p, axis=-1, keepdims=True)
            ctx = _dot(p.astype(_BF), c_s[b]) / l
            for k in range(nck):
                cabs_s[k, pl.ds(b, H, stride=B), :] = ctx[:, k * 128:(k + 1) * 128]

            for d in kv_copies(b, sk):
                d.wait()

            @pl.when(b + 2 < B)
            def _():
                for d in kv_copies(b + 2, sk):
                    d.start()

            @pl.when(b == B - 2)
            def _():
                cp(wo_hbm, wo_s, sk).start()

            @pl.when(b == B - 1)
            def _():
                bwo_copy(1, sk).start()

            first_half = lax.broadcasted_iota(jnp.int32, (8, 1), 0) < rep

            def kv_body(j, carry2):
                q8 = qb_s[pl.ds(b + j * 8 * B, 8, stride=B), :].astype(_BF)
                s0 = _dot_nt(q8, k_s[b, 2 * j])
                s1 = _dot_nt(q8, k_s[b, 2 * j + 1])
                sb = jnp.where(first_half, s0, s1)
                mb = jnp.max(sb, axis=-1, keepdims=True)
                pb = jnp.exp(sb - mb)
                lb = jnp.sum(pb, axis=-1, keepdims=True)
                pb = pb.astype(_BF)
                o0 = _dot(pb, v_s[b, 2 * j])
                o1 = _dot(pb, v_s[b, 2 * j + 1])
                ob = jnp.where(first_half, o0, o1) / lb
                ob_s[pl.ds(pl.multiple_of(b * Hq + j * 8, 8), 8), :] = ob
                return carry2

            lax.fori_loop(0, Hkv // 2, kv_body, 0)
            return carry

        lax.fori_loop(0, B, batch_body, 0)

        cp(wuv_hbm, wuv_s, 3).wait()
        bwo_copy(2, 3).start()

        def ctx_fn(h, w):
            rows = pl.ds(pl.multiple_of(h * B, B), B)
            lhs = jnp.concatenate([cabs_s[k, rows, :] for k in range(nck)], axis=1)
            ctx_s[rows, :] = _dot(lhs.astype(_BF), w)

        _head_pairs(wuv_s, Dc, H, ctx_fn)

        cp(wo_hbm, wo_s, 0).wait()

        def wo_body(g, acc):
            lhs = jnp.concatenate(
                [ctx_s[pl.ds(pl.multiple_of((g * 8 + r) * B, B), B), :] for r in range(8)],
                axis=1).astype(_BF)
            rows = pl.ds(pl.multiple_of(g * (8 * D), 8 * D), 8 * D)
            return acc + _dot(lhs, wo_s[rows, :])

        out_a = lax.fori_loop(0, H // 8, wo_body, jnp.zeros((B, M), _F32))

        out_b = jnp.zeros((B, M), _F32)
        for i, sem in enumerate((1, 2, 3)):
            bwo_copy(i, sem).wait()
            lo, hi = wo_parts[i]

            def bwo_step(h, acc):
                lhs = ob_s[pl.ds(h, B, stride=Hq), :].astype(_BF)
                rows = pl.ds(pl.multiple_of(h * Dh, Dh), Dh)
                return acc + _dot(lhs, bwo_s[rows, :])

            if hi - lo > 4:
                out_b = lax.fori_loop(lo, hi, bwo_step, out_b, unroll=2)
            else:
                for h in range(lo, hi):
                    out_b = bwo_step(h, out_b)

        out = gate * out_a + (1.0 - gate) * out_b
        o_ref[...] = out.astype(o_ref.dtype).reshape(B, Sq, M)

    any_spec = pl.BlockSpec(memory_space=pl.ANY)
    scratch = [
        pltpu.VMEM((B, Sq, M), _BF),
        pltpu.VMEM((M,), _BF),
        pltpu.VMEM((B, Sk, Dc), _BF),
        pltpu.VMEM((M * H, D), _BF),
        pltpu.VMEM((Dc * H, D), _BF),
        pltpu.VMEM((Dc * H, D), _BF),
        pltpu.VMEM((H * D, M), _BF),
        pltpu.VMEM((B, Hkv, W, Dh), _BF),
        pltpu.VMEM((B, Hkv, W, Dh), _BF),
        pltpu.VMEM((M, Hq * Dh), _BF),
        pltpu.VMEM((Hq * Dh, M), _BF),
        pltpu.VMEM((Hq * B, Dh), _F32),
        pltpu.VMEM((H * B, D), _F32),
        pltpu.VMEM((nck, H * B, 128), _F32),
        pltpu.VMEM((nck, H * B, 128), _F32),
        pltpu.VMEM((H * B, D), _F32),
        pltpu.VMEM((B * Hq, Dh), _F32),
        pltpu.SemaphoreType.DMA((4,)),
    ]
    return pl.pallas_call(
        kernel,
        out_shape=jax.ShapeDtypeStruct((B, Sq, M), A_x.dtype),
        in_specs=[any_spec] * 11,
        out_specs=pl.BlockSpec(memory_space=pltpu.VMEM),
        scratch_shapes=scratch,
        compiler_params=pltpu.CompilerParams(vmem_limit_bytes=110 * 2**20),
    )(A_x, A_c_kv, A_w_q.reshape(M * H, D), A_w_uk.reshape(Dc * H, D), A_w_uv.reshape(Dc * H, D),
      A_w_o.reshape(H * D, M), B_k_cache, B_v_cache, B_wq, B_wo, gate_w)
```

```python
import jax
import jax.numpy as jnp
from jax import lax
import jax.experimental.pallas as pl
import jax.experimental.pallas.tpu as pltpu

_BF = jnp.bfloat16
_F32 = jnp.float32
_NT = (((1,), (1,)), ((), ()))


def _dot(a, b):
    return jnp.dot(a, b, preferred_element_type=_F32)


def _dot_nt(a, b):
    return lax.dot_general(a, b, _NT, preferred_element_type=_F32)


def _head_pairs(w_ref, n_rows, n_heads, fn):
    w32 = w_ref.bitcast(jnp.uint32)
    npair = n_heads // 2
    grp = 4
    half = n_rows // 2
    span = n_rows * npair - (npair - grp)

    def body(jj, carry):
        sub = w32.at[pl.ds(pl.multiple_of(jj * grp, grp), span), :]
        for r in range(grp):
            ev = sub[pl.ds(r, half, stride=2 * npair), :]
            od = sub[pl.ds(r + npair, half, stride=2 * npair), :]
            lo = (ev & jnp.uint32(0xFFFF)) | (od << 16)
            hi = (ev >> 16) | (od & jnp.uint32(0xFFFF0000))
            h = 2 * (jj * grp + r)
            fn(h, pltpu.bitcast(lo, _BF))
            fn(h + 1, pltpu.bitcast(hi, _BF))
        return carry

    lax.fori_loop(0, npair // grp, body, 0)


@jax.jit
def pallas_gated_mix__compressed_kv_cla__sliding_block_cached__decode_kernel(
    A_x: jax.Array,
    A_c_kv: jax.Array,
    A_w_q: jax.Array,
    A_w_uk: jax.Array,
    A_w_uv: jax.Array,
    A_w_o: jax.Array,
    B_x: jax.Array,
    B_k_cache: jax.Array,
    B_v_cache: jax.Array,
    B_wq: jax.Array,
    B_wo: jax.Array,
    gate_w: jax.Array,
):
    del B_x
    B, Sq, M = A_x.shape
    Sk, Dc = A_c_kv.shape[1], A_c_kv.shape[2]
    H, D = A_w_q.shape[1], A_w_q.shape[2]
    Hq, Dh = 32, 128
    Hkv, SkB = B_k_cache.shape[1], B_k_cache.shape[2]
    W = min(4096, max(256, SkB // 4))
    rep = Hq // Hkv
    assert Sq == 1 and B == 8 and D == 128 and Dh == 128 and rep == 4 and H == Hq
    nck = Dc // 128
    scale_a = float(D) ** -0.5
    scale_b = float(Dh) ** -0.5
    wo_parts = ((0, 24), (24, 30), (30, 32))

    def kernel(x_hbm, c_hbm, wq_hbm, wuk_hbm, wuv_hbm, wo_hbm, k_hbm, v_hbm, bwq_hbm, bwo_hbm,
               gw_hbm, o_ref,
               x_s, gw_s, c_s, wq_s, wuk_s, wuv_s, wo_s, k_s, v_s, bwq_s, bwo_s,
               qb_s, qa_s, qabs_s, cabs_s, ctx_s, ob_s, sems):

        def cp(src, dst, s):
            return pltpu.make_async_copy(src, dst, sems.at[s])

        def c_copy(b, s):
            return cp(c_hbm.at[b], c_s.at[b], s)

        def kv_copies(b, s):
            return (cp(k_hbm.at[b, :, pl.ds(SkB - W, W), :], k_s.at[b], s),
                    cp(v_hbm.at[b, :, pl.ds(SkB - W, W), :], v_s.at[b], s))

        def bwo_copy(i, s):
            lo, hi = wo_parts[i]
            rows = pl.ds(lo * Dh, (hi - lo) * Dh)
            return cp(bwo_hbm.at[rows, :], bwo_s.at[rows, :], s)

        first = (cp(bwq_hbm, bwq_s, 0), cp(x_hbm, x_s, 0), cp(gw_hbm, gw_s, 0))
        for d in first:
            d.start()
        cp(wq_hbm, wq_s, 1).start()
        cp(wuk_hbm, wuk_s, 2).start()
        c_copy(0, 3).start()

        for d in first:
            d.wait()
        for d in kv_copies(0, 0):
            d.start()
        x = x_s[...]
        xf = x.astype(_F32)
        gate = jax.nn.sigmoid(
            jnp.sum(xf * gw_s[...].reshape(1, M).astype(_F32), axis=-1, keepdims=True))

        def qb_body(g, carry):
            cols = pl.ds(pl.multiple_of(g * (8 * Dh), 8 * Dh), 8 * Dh)
            q = _dot(x, bwq_s[:, cols]).astype(_BF).astype(_F32) * scale_b
            for r in range(8):
                row = pl.multiple_of((g * 8 + r) * B, B)
                qb_s[pl.ds(row, B), :] = q[:, r * Dh:(r + 1) * Dh]
            return carry

        lax.fori_loop(0, Hq // 8, qb_body, 0)

        cp(wq_hbm, wq_s, 1).wait()
        c_copy(1, 1).start()

        def qa_fn(h, w):
            qa_s[pl.ds(pl.multiple_of(h * B, B), B), :] = _dot(x, w)

        _head_pairs(wq_s, M, H, qa_fn)

        cp(wuk_hbm, wuk_s, 2).wait()
        for d in kv_copies(1, 2):
            d.start()

        def qabs_fn(h, w):
            rows = pl.ds(pl.multiple_of(h * B, B), B)
            r = _dot_nt(qa_s[rows, :].astype(_BF), w) * scale_a
            for k in range(nck):
                qabs_s[k, rows, :] = r[:, k * 128:(k + 1) * 128]

        _head_pairs(wuk_s, Dc, H, qabs_fn)

        def batch_body(b, carry):
            sc = jnp.where(b % 2 == 0, 3, 1)
            sk = jnp.where(b % 2 == 0, 0, 2)

            c_copy(b, sc).wait()

            @pl.when(b + 2 < B)
            def _():
                c_copy(b + 2, sc).start()

            @pl.when(b == B - 2)
            def _():
                cp(wuv_hbm, wuv_s, sc).start()

            @pl.when(b == B - 1)
            def _():
                bwo_copy(0, sc).start()

            q = jnp.concatenate([qabs_s[k, pl.ds(b, H, stride=B), :] for k in range(nck)],
                                axis=1).astype(_BF)
            c = c_s[b]
            s = _dot_nt(q, c)
            m = jnp.max(s, axis=-1, keepdims=True)
            p = jnp.exp(s - m)
            l = jnp.sum(p, axis=-1, keepdims=True)
            ctx = _dot(p.astype(_BF), c_s[b]) / l
            for k in range(nck):
                cabs_s[k, pl.ds(b, H, stride=B), :] = ctx[:, k * 128:(k + 1) * 128]

            for d in kv_copies(b, sk):
                d.wait()

            @pl.when(b + 2 < B)
            def _():
                for d in kv_copies(b + 2, sk):
                    d.start()

            @pl.when(b == B - 2)
            def _():
                cp(wo_hbm, wo_s, sk).start()

            @pl.when(b == B - 1)
            def _():
                bwo_copy(1, sk).start()

            first_half = lax.broadcasted_iota(jnp.int32, (8, 1), 0) < rep

            def kv_body(j, carry2):
                q8 = qb_s[pl.ds(b + j * 8 * B, 8, stride=B), :].astype(_BF)
                s0 = _dot_nt(q8, k_s[b, 2 * j])
                s1 = _dot_nt(q8, k_s[b, 2 * j + 1])
                sb = jnp.where(first_half, s0, s1)
                mb = jnp.max(sb, axis=-1, keepdims=True)
                pb = jnp.exp(sb - mb)
                lb = jnp.sum(pb, axis=-1, keepdims=True)
                pb = pb.astype(_BF)
                o0 = _dot(pb, v_s[b, 2 * j])
                o1 = _dot(pb, v_s[b, 2 * j + 1])
                ob = jnp.where(first_half, o0, o1) / lb
                ob_s[pl.ds(pl.multiple_of(b * Hq + j * 8, 8), 8), :] = ob
                return carry2

            lax.fori_loop(0, Hkv // 2, kv_body, 0)
            return carry

        lax.fori_loop(0, B, batch_body, 0)

        cp(wuv_hbm, wuv_s, 3).wait()
        bwo_copy(2, 3).start()

        def ctx_fn(h, w):
            rows = pl.ds(pl.multiple_of(h * B, B), B)
            lhs = jnp.concatenate([cabs_s[k, rows, :] for k in range(nck)], axis=1)
            ctx_s[rows, :] = _dot(lhs.astype(_BF), w)

        _head_pairs(wuv_s, Dc, H, ctx_fn)

        cp(wo_hbm, wo_s, 0).wait()

        def wo_body(g, acc):
            lhs = jnp.concatenate(
                [ctx_s[pl.ds(pl.multiple_of((g * 8 + r) * B, B), B), :] for r in range(8)],
                axis=1).astype(_BF)
            rows = pl.ds(pl.multiple_of(g * (8 * D), 8 * D), 8 * D)
            return acc + _dot(lhs, wo_s[rows, :])

        out_a = lax.fori_loop(0, H // 8, wo_body, jnp.zeros((B, M), _F32))

        out_b = jnp.zeros((B, M), _F32)
        for i, sem in enumerate((1, 2, 3)):
            bwo_copy(i, sem).wait()
            lo, hi = wo_parts[i]

            def bwo_step(h, acc):
                lhs = ob_s[pl.ds(h, B, stride=Hq), :].astype(_BF)
                rows = pl.ds(pl.multiple_of(h * Dh, Dh), Dh)
                return acc + _dot(lhs, bwo_s[rows, :])

            if hi - lo > 4:
                out_b = lax.fori_loop(lo, hi, bwo_step, out_b, unroll=2)
            else:
                for h in range(lo, hi):
                    out_b = bwo_step(h, out_b)

        out = gate * out_a + (1.0 - gate) * out_b
        o_ref[...] = out.astype(o_ref.dtype)

    any_spec = pl.BlockSpec(memory_space=pl.ANY)
    scratch = [
        pltpu.VMEM((B, M), _BF),
        pltpu.VMEM((M,), _BF),
        pltpu.VMEM((B, Sk, Dc), _BF),
        pltpu.VMEM((M * H, D), _BF),
        pltpu.VMEM((Dc * H, D), _BF),
        pltpu.VMEM((Dc * H, D), _BF),
        pltpu.VMEM((H * D, M), _BF),
        pltpu.VMEM((B, Hkv, W, Dh), _BF),
        pltpu.VMEM((B, Hkv, W, Dh), _BF),
        pltpu.VMEM((M, Hq * Dh), _BF),
        pltpu.VMEM((Hq * Dh, M), _BF),
        pltpu.VMEM((Hq * B, Dh), _F32),
        pltpu.VMEM((H * B, D), _F32),
        pltpu.VMEM((nck, H * B, 128), _F32),
        pltpu.VMEM((nck, H * B, 128), _F32),
        pltpu.VMEM((H * B, D), _F32),
        pltpu.VMEM((B * Hq, Dh), _F32),
        pltpu.SemaphoreType.DMA((4,)),
    ]
    return pl.pallas_call(
        kernel,
        out_shape=jax.ShapeDtypeStruct((B, M), A_x.dtype),
        in_specs=[any_spec] * 11,
        out_specs=pl.BlockSpec(memory_space=pltpu.VMEM),
        scratch_shapes=scratch,
        compiler_params=pltpu.CompilerParams(vmem_limit_bytes=110 * 2**20),
    )(A_x.reshape(B, M), A_c_kv, A_w_q.reshape(M * H, D), A_w_uk.reshape(Dc * H, D), A_w_uv.reshape(Dc * H, D),
      A_w_o.reshape(H * D, M), B_k_cache, B_v_cache, B_wq, B_wo, gate_w).reshape(B, Sq, M)
```

```python
import jax
import jax.numpy as jnp
from jax import lax
import jax.experimental.pallas as pl
import jax.experimental.pallas.tpu as pltpu

_BF = jnp.bfloat16
_F32 = jnp.float32
_NT = (((1,), (1,)), ((), ()))
_CHUNK_BYTES = 128 * 1024


def _dot(a, b):
    return jnp.dot(a, b, preferred_element_type=_F32)


def _dot_nt(a, b):
    return lax.dot_general(a, b, _NT, preferred_element_type=_F32)


def _head_pairs(w_ref, n_rows, n_heads, fn):
    w32 = w_ref.bitcast(jnp.uint32)
    npair = n_heads // 2
    grp = 4
    half = n_rows // 2
    span = n_rows * npair - (npair - grp)

    def body(jj, carry):
        sub = w32.at[pl.ds(pl.multiple_of(jj * grp, grp), span), :]
        for r in range(grp):
            ev = sub[pl.ds(r, half, stride=2 * npair), :]
            od = sub[pl.ds(r + npair, half, stride=2 * npair), :]
            lo = (ev & jnp.uint32(0xFFFF)) | (od << 16)
            hi = (ev >> 16) | (od & jnp.uint32(0xFFFF0000))
            h = 2 * (jj * grp + r)
            fn(h, pltpu.bitcast(lo, _BF))
            fn(h + 1, pltpu.bitcast(hi, _BF))
        return carry

    lax.fori_loop(0, npair // grp, body, 0)


@jax.jit
def pallas_gated_mix__compressed_kv_cla__sliding_block_cached__decode_kernel(
    A_x: jax.Array,
    A_c_kv: jax.Array,
    A_w_q: jax.Array,
    A_w_uk: jax.Array,
    A_w_uv: jax.Array,
    A_w_o: jax.Array,
    B_x: jax.Array,
    B_k_cache: jax.Array,
    B_v_cache: jax.Array,
    B_wq: jax.Array,
    B_wo: jax.Array,
    gate_w: jax.Array,
):
    del B_x
    B, Sq, M = A_x.shape
    Sk, Dc = A_c_kv.shape[1], A_c_kv.shape[2]
    H, D = A_w_q.shape[1], A_w_q.shape[2]
    Hq, Dh = 32, 128
    Hkv, SkB = B_k_cache.shape[1], B_k_cache.shape[2]
    W = min(4096, max(256, SkB // 4))
    rep = Hq // Hkv
    assert Sq == 1 and B == 8 and D == 128 and Dh == 128 and rep == 4 and H == Hq
    nck = Dc // 128
    scale_a = float(D) ** -0.5
    scale_b = float(Dh) ** -0.5
    wo_parts = ((0, 24), (24, 30), (30, 32))

    def kernel(x_hbm, c_hbm, wq_hbm, wuk_hbm, wuv_hbm, wo_hbm, k_hbm, v_hbm, bwq_hbm, bwo_hbm,
               gw_hbm, o_ref,
               x_s, gw_s, c_s, wq_s, wuk_s, wuv_s, wo_s, k_s, v_s, bwq_s, bwo_s,
               qb_s, qa_s, qabs_s, cabs_s, ctx_s, ob_s, sems):

        def cp(src, dst, s):
            return pltpu.make_async_copy(src, dst, sems.at[s])

        def start_rows(src, dst, s, lo, n_chunks, rows):
            def two(i, carry):
                for t in range(2):
                    sl = pl.ds(pl.multiple_of(lo + (2 * i + t) * rows, rows), rows)
                    cp(src.at[sl, :], dst.at[sl, :], s).start(priority=t)
                return carry
            lax.fori_loop(0, n_chunks // 2, two, 0)

        def start_whole(src, dst, s):
            rows = _CHUNK_BYTES // (2 * src.shape[1])
            start_rows(src, dst, s, 0, src.shape[0] // rows, rows)

        def c_copy(b, s):
            return cp(c_hbm.at[b], c_s.at[b], s)

        def c_start(b, s):
            start_whole(c_hbm.at[b], c_s.at[b], s)

        def kv_copies(b, s):
            return (cp(k_hbm.at[b, :, pl.ds(SkB - W, W), :], k_s.at[b], s),
                    cp(v_hbm.at[b, :, pl.ds(SkB - W, W), :], v_s.at[b], s))

        def kv_start(b, s):
            rows = _CHUNK_BYTES // (2 * Dh)

            def one_head(h, carry):
                for src, dst in ((k_hbm, k_s), (v_hbm, v_s)):
                    for t in range(W // rows):
                        cp(src.at[b, h, pl.ds(SkB - W + t * rows, rows), :],
                           dst.at[b, h, pl.ds(t * rows, rows), :], s).start(priority=t % 2)
                return carry
            lax.fori_loop(0, Hkv, one_head, 0)

        def bwo_copy(i, s):
            lo, hi = wo_parts[i]
            rows = pl.ds(lo * Dh, (hi - lo) * Dh)
            return cp(bwo_hbm.at[rows, :], bwo_s.at[rows, :], s)

        def bwo_start(i, s):
            lo, hi = wo_parts[i]
            start_rows(bwo_hbm, bwo_s, s, lo * Dh, hi - lo, Dh)

        start_whole(bwq_hbm, bwq_s, 0)
        first = (cp(bwq_hbm, bwq_s, 0), cp(x_hbm, x_s, 0), cp(gw_hbm, gw_s, 0))
        first[1].start()
        first[2].start()
        start_whole(wq_hbm, wq_s, 1)
        start_whole(wuk_hbm, wuk_s, 2)
        c_start(0, 3)

        for d in first:
            d.wait()
        kv_start(0, 0)
        x = x_s[...]
        xf = x.astype(_F32)
        gate = jax.nn.sigmoid(
            jnp.sum(xf * gw_s[...].reshape(1, M).astype(_F32), axis=-1, keepdims=True))

        def qb_body(g, carry):
            cols = pl.ds(pl.multiple_of(g * (8 * Dh), 8 * Dh), 8 * Dh)
            q = _dot(x, bwq_s[:, cols]).astype(_BF).astype(_F32) * scale_b
            for r in range(8):
                row = pl.multiple_of((g * 8 + r) * B, B)
                qb_s[pl.ds(row, B), :] = q[:, r * Dh:(r + 1) * Dh]
            return carry

        lax.fori_loop(0, Hq // 8, qb_body, 0)

        cp(wq_hbm, wq_s, 1).wait()
        c_start(1, 1)

        def qa_fn(h, w):
            qa_s[pl.ds(pl.multiple_of(h * B, B), B), :] = _dot(x, w)

        _head_pairs(wq_s, M, H, qa_fn)

        cp(wuk_hbm, wuk_s, 2).wait()
        kv_start(1, 2)

        def qabs_fn(h, w):
            rows = pl.ds(pl.multiple_of(h * B, B), B)
            r = _dot_nt(qa_s[rows, :].astype(_BF), w) * scale_a
            for k in range(nck):
                qabs_s[k, rows, :] = r[:, k * 128:(k + 1) * 128]

        _head_pairs(wuk_s, Dc, H, qabs_fn)

        def batch_body(b, carry):
            sc = jnp.where(b % 2 == 0, 3, 1)
            sk = jnp.where(b % 2 == 0, 0, 2)

            c_copy(b, sc).wait()

            @pl.when(b + 2 < B)
            def _():
                c_start(b + 2, sc)

            @pl.when(b == B - 2)
            def _():
                start_whole(wuv_hbm, wuv_s, sc)

            @pl.when(b == B - 1)
            def _():
                bwo_start(0, sc)

            q = jnp.concatenate([qabs_s[k, pl.ds(b, H, stride=B), :] for k in range(nck)],
                                axis=1).astype(_BF)
            c = c_s[b]
            s = _dot_nt(q, c)
            m = jnp.max(s, axis=-1, keepdims=True)
            p = jnp.exp(s - m)
            l = jnp.sum(p, axis=-1, keepdims=True)
            ctx = _dot(p.astype(_BF), c_s[b]) / l
            for k in range(nck):
                cabs_s[k, pl.ds(b, H, stride=B), :] = ctx[:, k * 128:(k + 1) * 128]

            for d in kv_copies(b, sk):
                d.wait()

            @pl.when(b + 2 < B)
            def _():
                kv_start(b + 2, sk)

            @pl.when(b == B - 2)
            def _():
                start_whole(wo_hbm, wo_s, sk)

            @pl.when(b == B - 1)
            def _():
                bwo_start(1, sk)

            first_half = lax.broadcasted_iota(jnp.int32, (8, 1), 0) < rep

            def kv_body(j, carry2):
                q8 = qb_s[pl.ds(b + j * 8 * B, 8, stride=B), :].astype(_BF)
                s0 = _dot_nt(q8, k_s[b, 2 * j])
                s1 = _dot_nt(q8, k_s[b, 2 * j + 1])
                sb = jnp.where(first_half, s0, s1)
                mb = jnp.max(sb, axis=-1, keepdims=True)
                pb = jnp.exp(sb - mb)
                lb = jnp.sum(pb, axis=-1, keepdims=True)
                pb = pb.astype(_BF)
                o0 = _dot(pb, v_s[b, 2 * j])
                o1 = _dot(pb, v_s[b, 2 * j + 1])
                ob = jnp.where(first_half, o0, o1) / lb
                ob_s[pl.ds(pl.multiple_of(b * Hq + j * 8, 8), 8), :] = ob
                return carry2

            lax.fori_loop(0, Hkv // 2, kv_body, 0)
            return carry

        lax.fori_loop(0, B, batch_body, 0)

        cp(wuv_hbm, wuv_s, 3).wait()
        bwo_start(2, 3)

        def ctx_fn(h, w):
            rows = pl.ds(pl.multiple_of(h * B, B), B)
            lhs = jnp.concatenate([cabs_s[k, rows, :] for k in range(nck)], axis=1)
            ctx_s[rows, :] = _dot(lhs.astype(_BF), w)

        _head_pairs(wuv_s, Dc, H, ctx_fn)

        cp(wo_hbm, wo_s, 0).wait()

        def wo_body(g, acc):
            lhs = jnp.concatenate(
                [ctx_s[pl.ds(pl.multiple_of((g * 8 + r) * B, B), B), :] for r in range(8)],
                axis=1).astype(_BF)
            rows = pl.ds(pl.multiple_of(g * (8 * D), 8 * D), 8 * D)
            return acc + _dot(lhs, wo_s[rows, :])

        out_a = lax.fori_loop(0, H // 8, wo_body, jnp.zeros((B, M), _F32))

        out_b = jnp.zeros((B, M), _F32)
        for i, sem in enumerate((1, 2, 3)):
            bwo_copy(i, sem).wait()
            lo, hi = wo_parts[i]

            def bwo_step(h, acc):
                lhs = ob_s[pl.ds(h, B, stride=Hq), :].astype(_BF)
                rows = pl.ds(pl.multiple_of(h * Dh, Dh), Dh)
                return acc + _dot(lhs, bwo_s[rows, :])

            if hi - lo > 4:
                out_b = lax.fori_loop(lo, hi, bwo_step, out_b, unroll=2)
            else:
                for h in range(lo, hi):
                    out_b = bwo_step(h, out_b)

        out = gate * out_a + (1.0 - gate) * out_b
        o_ref[...] = out.astype(o_ref.dtype)

    any_spec = pl.BlockSpec(memory_space=pl.ANY)
    scratch = [
        pltpu.VMEM((B, M), _BF),
        pltpu.VMEM((M,), _BF),
        pltpu.VMEM((B, Sk, Dc), _BF),
        pltpu.VMEM((M * H, D), _BF),
        pltpu.VMEM((Dc * H, D), _BF),
        pltpu.VMEM((Dc * H, D), _BF),
        pltpu.VMEM((H * D, M), _BF),
        pltpu.VMEM((B, Hkv, W, Dh), _BF),
        pltpu.VMEM((B, Hkv, W, Dh), _BF),
        pltpu.VMEM((M, Hq * Dh), _BF),
        pltpu.VMEM((Hq * Dh, M), _BF),
        pltpu.VMEM((Hq * B, Dh), _F32),
        pltpu.VMEM((H * B, D), _F32),
        pltpu.VMEM((nck, H * B, 128), _F32),
        pltpu.VMEM((nck, H * B, 128), _F32),
        pltpu.VMEM((H * B, D), _F32),
        pltpu.VMEM((B * Hq, Dh), _F32),
        pltpu.SemaphoreType.DMA((4,)),
    ]
    return pl.pallas_call(
        kernel,
        out_shape=jax.ShapeDtypeStruct((B, M), A_x.dtype),
        in_specs=[any_spec] * 11,
        out_specs=pl.BlockSpec(memory_space=pltpu.VMEM),
        scratch_shapes=scratch,
        compiler_params=pltpu.CompilerParams(vmem_limit_bytes=110 * 2**20),
    )(A_x.reshape(B, M), A_c_kv, A_w_q.reshape(M * H, D), A_w_uk.reshape(Dc * H, D), A_w_uv.reshape(Dc * H, D),
      A_w_o.reshape(H * D, M), B_k_cache, B_v_cache, B_wq, B_wo, gate_w).reshape(B, Sq, M)
```

```python
import jax
import jax.numpy as jnp
from jax import lax
import jax.experimental.pallas as pl
import jax.experimental.pallas.tpu as pltpu

_BF = jnp.bfloat16
_F32 = jnp.float32
_NT = (((1,), (1,)), ((), ()))
_CHUNK_BYTES = 128 * 1024
_WO_PARTS = ((0, 16, 8), (16, 24, 4), (24, 28, 4), (28, 30, 2), (30, 32, 2))


def _dot(a, b):
    return jnp.dot(a, b, preferred_element_type=_F32)


def _dot_nt(a, b):
    return lax.dot_general(a, b, _NT, preferred_element_type=_F32)


def _for_each_head(w_ref, n_rows, n_heads, fn):
    w32 = w_ref.bitcast(jnp.uint32)
    npair = n_heads // 2
    grp = 4
    half = n_rows // 2
    span = n_rows * npair - (npair - grp)

    def body(jj, carry):
        sub = w32.at[pl.ds(pl.multiple_of(jj * grp, grp), span), :]
        for r in range(grp):
            ev = sub[pl.ds(r, half, stride=2 * npair), :]
            od = sub[pl.ds(r + npair, half, stride=2 * npair), :]
            lo = (ev & jnp.uint32(0xFFFF)) | (od << 16)
            hi = (ev >> 16) | (od & jnp.uint32(0xFFFF0000))
            h = 2 * (jj * grp + r)
            fn(h, pltpu.bitcast(lo, _BF))
            fn(h + 1, pltpu.bitcast(hi, _BF))
        return carry

    lax.fori_loop(0, npair // grp, body, 0)


@jax.jit
def pallas_gated_mix__compressed_kv_cla__sliding_block_cached__decode_kernel(
    A_x: jax.Array,
    A_c_kv: jax.Array,
    A_w_q: jax.Array,
    A_w_uk: jax.Array,
    A_w_uv: jax.Array,
    A_w_o: jax.Array,
    B_x: jax.Array,
    B_k_cache: jax.Array,
    B_v_cache: jax.Array,
    B_wq: jax.Array,
    B_wo: jax.Array,
    gate_w: jax.Array,
):
    del B_x
    B, Sq, M = A_x.shape
    Sk, Dc = A_c_kv.shape[1], A_c_kv.shape[2]
    H, D = A_w_q.shape[1], A_w_q.shape[2]
    Hq, Dh = 32, 128
    Hkv, SkB = B_k_cache.shape[1], B_k_cache.shape[2]
    W = min(4096, max(256, SkB // 4))
    rep = Hq // Hkv
    assert Sq == 1 and B == 8 and D == 128 and Dh == 128 and rep == 4 and H == Hq
    nck = Dc // 128
    scale_a = float(D) ** -0.5
    scale_b = float(Dh) ** -0.5
    n_parts = len(_WO_PARTS)

    def kernel(x_hbm, c_hbm, wq_hbm, wuk_hbm, wuv_hbm, wo_hbm, k_hbm, v_hbm, bwq_hbm, bwo_hbm,
               gw_hbm, o_ref,
               x_s, gw_s, c_s, wq_s, wuk_s, wuv_s, wo_s, k_s, v_s, bwq_s, bwo_s,
               qb_s, qa_s, qabs_s, cabs_s, ctx_s, ob_s, obl_s, sems):

        def cp(src, dst, s):
            return pltpu.make_async_copy(src, dst, sems.at[s])

        def start_rows(src, dst, s, lo, n_chunks, rows):
            def two(i, carry):
                for t in range(2):
                    sl = pl.ds(pl.multiple_of(lo + (2 * i + t) * rows, rows), rows)
                    cp(src.at[sl, :], dst.at[sl, :], s).start(priority=t)
                return carry
            lax.fori_loop(0, n_chunks // 2, two, 0)

        def start_whole(src, dst, s):
            rows = _CHUNK_BYTES // (2 * src.shape[1])
            start_rows(src, dst, s, 0, src.shape[0] // rows, rows)

        def kv_start(b, s):
            rows = _CHUNK_BYTES // (2 * Dh)

            def one_head(h, carry):
                for src, dst in ((k_hbm, k_s), (v_hbm, v_s)):
                    for t in range(W // rows):
                        cp(src.at[b, h, pl.ds(SkB - W + t * rows, rows), :],
                           dst.at[b, h, pl.ds(t * rows, rows), :], s).start(priority=t % 2)
                return carry
            lax.fori_loop(0, Hkv, one_head, 0)

        def bwo_start(i):
            lo, hi, _ = _WO_PARTS[i]
            if (hi - lo) % 2 == 0 and hi - lo > 4:
                start_rows(bwo_hbm, bwo_s, i, lo * Dh, hi - lo, Dh)
            else:
                for h in range(lo, hi):
                    sl = pl.ds(h * Dh, Dh)
                    cp(bwo_hbm.at[sl, :], bwo_s.at[sl, :], i).start(priority=h % 2)

        def kv_wait(b, s):
            cp(k_hbm.at[b, :, pl.ds(SkB - W, W), :], k_s.at[b], s).wait()
            cp(v_hbm.at[b, :, pl.ds(SkB - W, W), :], v_s.at[b], s).wait()

        def bwo_wait(i):
            lo, hi, _ = _WO_PARTS[i]
            rows = pl.ds(lo * Dh, (hi - lo) * Dh)
            cp(bwo_hbm.at[rows, :], bwo_s.at[rows, :], i).wait()

        start_whole(bwq_hbm, bwq_s, 0)
        cp(x_hbm, x_s, 0).start()
        cp(gw_hbm, gw_s, 0).start()
        start_whole(wq_hbm, wq_s, 1)
        start_whole(wuk_hbm, wuk_s, 2)

        cp(bwq_hbm, bwq_s, 0).wait()
        cp(x_hbm, x_s, 0).wait()
        cp(gw_hbm, gw_s, 0).wait()
        start_whole(c_hbm.at[0], c_s.at[0], 0)

        x = x_s[...]
        gate = jax.nn.sigmoid(jnp.sum(
            x.astype(_F32) * gw_s[...].reshape(1, M).astype(_F32), axis=-1, keepdims=True))

        def qb_body(g, carry):
            cols = pl.ds(pl.multiple_of(g * (8 * Dh), 8 * Dh), 8 * Dh)
            q = _dot(x, bwq_s[:, cols]).astype(_BF).astype(_F32) * scale_b
            for r in range(8):
                row = pl.multiple_of((g * 8 + r) * B, B)
                qb_s[pl.ds(row, B), :] = q[:, r * Dh:(r + 1) * Dh]
            return carry

        lax.fori_loop(0, Hq // 8, qb_body, 0)

        cp(wq_hbm, wq_s, 1).wait()
        kv_start(0, 1)

        def qa_fn(h, w):
            qa_s[pl.ds(pl.multiple_of(h * B, B), B), :] = _dot(x, w)

        _for_each_head(wq_s, M, H, qa_fn)

        cp(wuk_hbm, wuk_s, 2).wait()
        start_whole(c_hbm.at[1], c_s.at[1], 2)

        def qabs_fn(h, w):
            rows = pl.ds(pl.multiple_of(h * B, B), B)
            r = _dot_nt(qa_s[rows, :].astype(_BF), w) * scale_a
            for k in range(nck):
                qabs_s[k, rows, :] = r[:, k * 128:(k + 1) * 128]

        _for_each_head(wuk_s, Dc, H, qabs_fn)

        def batch_body(b, carry):
            sc = (2 * b) % 3
            sk = (2 * b + 1) % 3

            cp(c_hbm.at[b], c_s.at[b], sc).wait()

            @pl.when(b < B - 1)
            def _():
                kv_start(b + 1, sc)

            @pl.when(b == B - 1)
            def _():
                start_whole(wo_hbm, wo_s, sc)

            q = jnp.concatenate([qabs_s[k, pl.ds(b, H, stride=B), :] for k in range(nck)],
                                axis=1).astype(_BF)
            s = _dot_nt(q, c_s[b])
            m = jnp.max(s, axis=-1, keepdims=True)
            p = jnp.exp(s - m)
            l = jnp.sum(p, axis=-1, keepdims=True)
            ctx = _dot(p.astype(_BF), c_s[b]) / l
            for k in range(nck):
                cabs_s[k, pl.ds(b, H, stride=B), :] = ctx[:, k * 128:(k + 1) * 128]

            kv_wait(b, sk)

            @pl.when(b < B - 2)
            def _():
                start_whole(c_hbm.at[b + 2], c_s.at[b + 2], sk)

            @pl.when(b == B - 2)
            def _():
                start_whole(wuv_hbm, wuv_s, sk)

            @pl.when(b == B - 1)
            def _():
                bwo_start(0)

            first = lax.broadcasted_iota(jnp.int32, (8, 1), 0) < rep

            def kv_body(j, carry2):
                q8 = qb_s[pl.ds(b + j * 8 * B, 8, stride=B), :].astype(_BF)
                s0 = _dot_nt(q8, k_s[b, 2 * j])
                s1 = _dot_nt(q8, k_s[b, 2 * j + 1])
                sb = jnp.where(first, s0, s1)
                mb = jnp.max(sb, axis=-1, keepdims=True)
                pb = jnp.exp(sb - mb)
                lb = jnp.sum(pb, axis=-1, keepdims=True)
                pb = pb.astype(_BF)
                o0 = _dot(pb, v_s[b, 2 * j])
                o1 = _dot(pb, v_s[b, 2 * j + 1])
                ob_s[pl.ds(b + j * 8 * B, 8, stride=B), :] = jnp.where(first, o0, o1) / lb
                return carry2

            lax.fori_loop(0, Hkv // 2, kv_body, 0)
            return carry

        lax.fori_loop(0, B, batch_body, 0)
        obl_s[...] = jnp.concatenate(
            [ob_s[h * B:(h + 1) * B, :] for h in range(Hq)], axis=1).astype(_BF)

        cp(wuv_hbm, wuv_s, 1).wait()
        bwo_start(1)

        def ctx_fn(h, w):
            rows = pl.ds(pl.multiple_of(h * B, B), B)
            lhs = jnp.concatenate([cabs_s[k, rows, :] for k in range(nck)], axis=1)
            ctx_s[rows, :] = _dot(lhs.astype(_BF), w)

        _for_each_head(wuv_s, Dc, H, ctx_fn)

        cp(wo_hbm, wo_s, 2).wait()
        for i in range(2, n_parts):
            bwo_start(i)

        def wo_body(g, acc):
            lhs = jnp.concatenate(
                [ctx_s[pl.ds(pl.multiple_of((g * 8 + r) * B, B), B), :] for r in range(8)],
                axis=1).astype(_BF)
            rows = pl.ds(pl.multiple_of(g * (8 * D), 8 * D), 8 * D)
            return acc + _dot(lhs, wo_s[rows, :])

        out_a = lax.fori_loop(0, H // 8, wo_body, jnp.zeros((B, M), _F32))

        out_b = jnp.zeros((B, M), _F32)
        for i, (lo, hi, g) in enumerate(_WO_PARTS):
            bwo_wait(i)
            n_it = (hi - lo) // g

            def bwo_step(t, acc, lo=lo, g=g):
                rows = pl.ds(pl.multiple_of((lo + t * g) * Dh, Dh), g * Dh)
                return acc + _dot(obl_s[:, rows], bwo_s[rows, :])

            if n_it > 1:
                out_b = lax.fori_loop(0, n_it, bwo_step, out_b)
            else:
                out_b = out_b + _dot(obl_s[:, lo * Dh:hi * Dh], bwo_s[lo * Dh:hi * Dh, :])

        out = gate * out_a + (1.0 - gate) * out_b
        o_ref[...] = out.astype(o_ref.dtype)

    any_spec = pl.BlockSpec(memory_space=pl.ANY)
    scratch = [
        pltpu.VMEM((B, M), _BF),
        pltpu.VMEM((M,), _BF),
        pltpu.VMEM((B, Sk, Dc), _BF),
        pltpu.VMEM((M * H, D), _BF),
        pltpu.VMEM((Dc * H, D), _BF),
        pltpu.VMEM((Dc * H, D), _BF),
        pltpu.VMEM((H * D, M), _BF),
        pltpu.VMEM((B, Hkv, W, Dh), _BF),
        pltpu.VMEM((B, Hkv, W, Dh), _BF),
        pltpu.VMEM((M, Hq * Dh), _BF),
        pltpu.VMEM((Hq * Dh, M), _BF),
        pltpu.VMEM((Hq * B, Dh), _F32),
        pltpu.VMEM((H * B, D), _F32),
        pltpu.VMEM((nck, H * B, 128), _F32),
        pltpu.VMEM((nck, H * B, 128), _F32),
        pltpu.VMEM((H * B, D), _F32),
        pltpu.VMEM((Hq * B, Dh), _F32),
        pltpu.VMEM((B, Hq * Dh), _BF),
        pltpu.SemaphoreType.DMA((max(3, n_parts),)),
    ]
    out = pl.pallas_call(
        kernel,
        out_shape=jax.ShapeDtypeStruct((B, M), A_x.dtype),
        in_specs=[any_spec] * 11,
        out_specs=pl.BlockSpec(memory_space=pltpu.VMEM),
        scratch_shapes=scratch,
        compiler_params=pltpu.CompilerParams(vmem_limit_bytes=110 * 2**20),
    )(A_x.reshape(B, M), A_c_kv, A_w_q.reshape(M * H, D), A_w_uk.reshape(Dc * H, D),
      A_w_uv.reshape(Dc * H, D), A_w_o.reshape(H * D, M), B_k_cache, B_v_cache, B_wq, B_wo, gate_w)
    return out.reshape(B, Sq, M)
```

```python
import jax
import jax.numpy as jnp
from jax import lax
import jax.experimental.pallas as pl
import jax.experimental.pallas.tpu as pltpu

_BF = jnp.bfloat16
_F32 = jnp.float32
_NT = (((1,), (1,)), ((), ()))
_CHUNK_BYTES = 128 * 1024
_WO_PARTS = ((0, 16, 8), (16, 24, 4), (24, 28, 4), (28, 30, 2), (30, 32, 2))


def _dot(a, b):
    return jnp.dot(a, b, preferred_element_type=_F32)


def _dot_nt(a, b):
    return lax.dot_general(a, b, _NT, preferred_element_type=_F32)


def _for_each_head(w_ref, n_rows, n_heads, fn):
    w32 = w_ref.bitcast(jnp.uint32)
    npair = n_heads // 2
    grp = 4
    half = n_rows // 2
    span = n_rows * npair - (npair - grp)

    def body(jj, carry):
        sub = w32.at[pl.ds(pl.multiple_of(jj * grp, grp), span), :]
        for r in range(grp):
            ev = sub[pl.ds(r, half, stride=2 * npair), :]
            od = sub[pl.ds(r + npair, half, stride=2 * npair), :]
            lo = (ev & jnp.uint32(0xFFFF)) | (od << 16)
            hi = (ev >> 16) | (od & jnp.uint32(0xFFFF0000))
            h = 2 * (jj * grp + r)
            fn(h, pltpu.bitcast(lo, _BF))
            fn(h + 1, pltpu.bitcast(hi, _BF))
        return carry

    lax.fori_loop(0, npair // grp, body, 0)


@jax.jit
def pallas_gated_mix__compressed_kv_cla__sliding_block_cached__decode_kernel(
    A_x: jax.Array,
    A_c_kv: jax.Array,
    A_w_q: jax.Array,
    A_w_uk: jax.Array,
    A_w_uv: jax.Array,
    A_w_o: jax.Array,
    B_x: jax.Array,
    B_k_cache: jax.Array,
    B_v_cache: jax.Array,
    B_wq: jax.Array,
    B_wo: jax.Array,
    gate_w: jax.Array,
):
    del B_x
    B, Sq, M = A_x.shape
    Sk, Dc = A_c_kv.shape[1], A_c_kv.shape[2]
    H, D = A_w_q.shape[1], A_w_q.shape[2]
    Hq, Dh = 32, 128
    Hkv, SkB = B_k_cache.shape[1], B_k_cache.shape[2]
    W = min(4096, max(256, SkB // 4))
    rep = Hq // Hkv
    assert Sq == 1 and B == 8 and D == 128 and Dh == 128 and rep == 4 and H == Hq
    nck = Dc // 128
    scale_a = float(D) ** -0.5
    scale_b = float(Dh) ** -0.5
    n_parts = len(_WO_PARTS)

    def kernel(x_hbm, c_hbm, wq_hbm, wuk_hbm, wuv_hbm, wo_hbm, k_hbm, v_hbm, bwq_hbm, bwo_hbm,
               gw_hbm, o_ref,
               x_s, gw_s, c_s, wq_s, wuk_s, wuv_s, wo_s, k_s, v_s, bwq_s, bwo_s,
               qb_s, qa_s, qabs_s, cabs_s, ctx_s, ob_s, obl_s, sems):

        def cp(src, dst, s):
            return pltpu.make_async_copy(src, dst, sems.at[s])

        def start_rows(src, dst, s, lo, n_chunks, rows):
            def two(i, carry):
                for t in range(2):
                    sl = pl.ds(pl.multiple_of(lo + (2 * i + t) * rows, rows), rows)
                    cp(src.at[sl, :], dst.at[sl, :], s).start(priority=t)
                return carry
            lax.fori_loop(0, n_chunks // 2, two, 0)

        def start_whole(src, dst, s):
            rows = _CHUNK_BYTES // (2 * src.shape[1])
            start_rows(src, dst, s, 0, src.shape[0] // rows, rows)

        def kv_start(b, s):
            rows = _CHUNK_BYTES // (2 * Dh)

            def one_head(h, carry):
                for src, dst in ((k_hbm, k_s), (v_hbm, v_s)):
                    for t in range(W // rows):
                        cp(src.at[b, h, pl.ds(SkB - W + t * rows, rows), :],
                           dst.at[b, h, pl.ds(t * rows, rows), :], s).start(priority=t % 2)
                return carry
            lax.fori_loop(0, Hkv, one_head, 0)

        def bwo_start(i):
            lo, hi, _ = _WO_PARTS[i]
            if (hi - lo) % 2 == 0 and hi - lo > 4:
                start_rows(bwo_hbm, bwo_s, i % 3, lo * Dh, hi - lo, Dh)
            else:
                for h in range(lo, hi):
                    sl = pl.ds(h * Dh, Dh)
                    cp(bwo_hbm.at[sl, :], bwo_s.at[sl, :], i % 3).start(priority=1)

        def kv_wait(b, s):
            cp(k_hbm.at[b, :, pl.ds(SkB - W, W), :], k_s.at[b], s).wait()
            cp(v_hbm.at[b, :, pl.ds(SkB - W, W), :], v_s.at[b], s).wait()

        def bwo_wait(i):
            lo, hi, _ = _WO_PARTS[i]
            rows = pl.ds(lo * Dh, (hi - lo) * Dh)
            cp(bwo_hbm.at[rows, :], bwo_s.at[rows, :], i % 3).wait()

        start_whole(bwq_hbm, bwq_s, 0)
        cp(x_hbm, x_s, 0).start()
        cp(gw_hbm, gw_s, 0).start()
        start_whole(wq_hbm, wq_s, 1)
        start_whole(wuk_hbm, wuk_s, 2)

        cp(bwq_hbm, bwq_s, 0).wait()
        cp(x_hbm, x_s, 0).wait()
        cp(gw_hbm, gw_s, 0).wait()
        start_whole(c_hbm.at[0], c_s.at[0], 0)

        x = x_s[...]
        gate = jax.nn.sigmoid(jnp.sum(
            x.astype(_F32) * gw_s[...].reshape(1, M).astype(_F32), axis=-1, keepdims=True))

        def qb_body(g, carry):
            cols = pl.ds(pl.multiple_of(g * (8 * Dh), 8 * Dh), 8 * Dh)
            q = _dot(x, bwq_s[:, cols]).astype(_BF).astype(_F32) * scale_b
            for r in range(8):
                row = pl.multiple_of((g * 8 + r) * B, B)
                qb_s[pl.ds(row, B), :] = q[:, r * Dh:(r + 1) * Dh]
            return carry

        lax.fori_loop(0, Hq // 8, qb_body, 0)

        cp(wq_hbm, wq_s, 1).wait()
        kv_start(0, 1)

        def qa_fn(h, w):
            qa_s[pl.ds(pl.multiple_of(h * B, B), B), :] = _dot(x, w)

        _for_each_head(wq_s, M, H, qa_fn)

        cp(wuk_hbm, wuk_s, 2).wait()
        start_whole(c_hbm.at[1], c_s.at[1], 2)

        def qabs_fn(h, w):
            rows = pl.ds(pl.multiple_of(h * B, B), B)
            r = _dot_nt(qa_s[rows, :].astype(_BF), w) * scale_a
            for k in range(nck):
                qabs_s[k, rows, :] = r[:, k * 128:(k + 1) * 128]

        _for_each_head(wuk_s, Dc, H, qabs_fn)

        def batch_body(b, carry):
            sc = (2 * b) % 3
            sk = (2 * b + 1) % 3

            cp(c_hbm.at[b], c_s.at[b], sc).wait()

            @pl.when(b < B - 1)
            def _():
                kv_start(b + 1, sc)

            @pl.when(b == B - 1)
            def _():
                start_whole(wo_hbm, wo_s, sc)

            q = jnp.concatenate([qabs_s[k, pl.ds(b, H, stride=B), :] for k in range(nck)],
                                axis=1).astype(_BF)
            s = _dot_nt(q, c_s[b])
            m = jnp.max(s, axis=-1, keepdims=True)
            p = jnp.exp(s - m)
            l = jnp.sum(p, axis=-1, keepdims=True)
            ctx = _dot(p.astype(_BF), c_s[b]) / l
            for k in range(nck):
                cabs_s[k, pl.ds(b, H, stride=B), :] = ctx[:, k * 128:(k + 1) * 128]

            kv_wait(b, sk)

            @pl.when(b < B - 2)
            def _():
                start_whole(c_hbm.at[b + 2], c_s.at[b + 2], sk)

            @pl.when(b == B - 2)
            def _():
                start_whole(wuv_hbm, wuv_s, sk)

            @pl.when(b == B - 1)
            def _():
                bwo_start(0)

            first = lax.broadcasted_iota(jnp.int32, (8, 1), 0) < rep

            def kv_body(j, carry2):
                q8 = qb_s[pl.ds(b + j * 8 * B, 8, stride=B), :].astype(_BF)
                s0 = _dot_nt(q8, k_s[b, 2 * j])
                s1 = _dot_nt(q8, k_s[b, 2 * j + 1])
                sb = jnp.where(first, s0, s1)
                mb = jnp.max(sb, axis=-1, keepdims=True)
                pb = jnp.exp(sb - mb)
                lb = jnp.sum(pb, axis=-1, keepdims=True)
                pb = pb.astype(_BF)
                o0 = _dot(pb, v_s[b, 2 * j])
                o1 = _dot(pb, v_s[b, 2 * j + 1])
                ob_s[pl.ds(b + j * 8 * B, 8, stride=B), :] = jnp.where(first, o0, o1) / lb
                return carry2

            lax.fori_loop(0, Hkv // 2, kv_body, 0)
            return carry

        lax.fori_loop(0, B, batch_body, 0)
        obl_s[...] = jnp.concatenate(
            [ob_s[h * B:(h + 1) * B, :] for h in range(Hq)], axis=1).astype(_BF)

        cp(wuv_hbm, wuv_s, 1).wait()
        bwo_start(1)

        def ctx_fn(h, w):
            rows = pl.ds(pl.multiple_of(h * B, B), B)
            lhs = jnp.concatenate([cabs_s[k, rows, :] for k in range(nck)], axis=1)
            ctx_s[rows, :] = _dot(lhs.astype(_BF), w)

        _for_each_head(wuv_s, Dc, H, ctx_fn)

        cp(wo_hbm, wo_s, 2).wait()
        bwo_start(2)

        def wo_body(g, acc):
            lhs = jnp.concatenate(
                [ctx_s[pl.ds(pl.multiple_of((g * 8 + r) * B, B), B), :] for r in range(8)],
                axis=1).astype(_BF)
            rows = pl.ds(pl.multiple_of(g * (8 * D), 8 * D), 8 * D)
            return acc + _dot(lhs, wo_s[rows, :])

        out_a = lax.fori_loop(0, H // 8, wo_body, jnp.zeros((B, M), _F32))

        out_b = jnp.zeros((B, M), _F32)
        for i, (lo, hi, g) in enumerate(_WO_PARTS):
            bwo_wait(i)
            if i + 3 < n_parts:
                bwo_start(i + 3)
            n_it = (hi - lo) // g

            def bwo_step(t, acc, lo=lo, g=g):
                rows = pl.ds(pl.multiple_of((lo + t * g) * Dh, Dh), g * Dh)
                return acc + _dot(obl_s[:, rows], bwo_s[rows, :])

            if n_it > 1:
                out_b = lax.fori_loop(0, n_it, bwo_step, out_b)
            else:
                out_b = out_b + _dot(obl_s[:, lo * Dh:hi * Dh], bwo_s[lo * Dh:hi * Dh, :])

        out = gate * out_a + (1.0 - gate) * out_b
        o_ref[...] = out.astype(o_ref.dtype)

    any_spec = pl.BlockSpec(memory_space=pl.ANY)
    scratch = [
        pltpu.VMEM((B, M), _BF),
        pltpu.VMEM((M,), _BF),
        pltpu.VMEM((B, Sk, Dc), _BF),
        pltpu.VMEM((M * H, D), _BF),
        pltpu.VMEM((Dc * H, D), _BF),
        pltpu.VMEM((Dc * H, D), _BF),
        pltpu.VMEM((H * D, M), _BF),
        pltpu.VMEM((B, Hkv, W, Dh), _BF),
        pltpu.VMEM((B, Hkv, W, Dh), _BF),
        pltpu.VMEM((M, Hq * Dh), _BF),
        pltpu.VMEM((Hq * Dh, M), _BF),
        pltpu.VMEM((Hq * B, Dh), _F32),
        pltpu.VMEM((H * B, D), _F32),
        pltpu.VMEM((nck, H * B, 128), _F32),
        pltpu.VMEM((nck, H * B, 128), _F32),
        pltpu.VMEM((H * B, D), _F32),
        pltpu.VMEM((Hq * B, Dh), _F32),
        pltpu.VMEM((B, Hq * Dh), _BF),
        pltpu.SemaphoreType.DMA((3,)),
    ]
    out = pl.pallas_call(
        kernel,
        out_shape=jax.ShapeDtypeStruct((B, M), A_x.dtype),
        in_specs=[any_spec] * 11,
        out_specs=pl.BlockSpec(memory_space=pltpu.VMEM),
        scratch_shapes=scratch,
        compiler_params=pltpu.CompilerParams(vmem_limit_bytes=110 * 2**20),
    )(A_x.reshape(B, M), A_c_kv, A_w_q.reshape(M * H, D), A_w_uk.reshape(Dc * H, D),
      A_w_uv.reshape(Dc * H, D), A_w_o.reshape(H * D, M), B_k_cache, B_v_cache, B_wq, B_wo, gate_w)
    return out.reshape(B, Sq, M)
```

```python
import jax
import jax.numpy as jnp
from jax import lax
import jax.experimental.pallas as pl
import jax.experimental.pallas.tpu as pltpu

_BF = jnp.bfloat16
_F32 = jnp.float32
_NT = (((1,), (1,)), ((), ()))
_G = 4
_UNIT_BYTES = 1 << 20
_DESC_BYTES = 32 << 10
_REGIONS = 4


def _dot(a, b):
    return jnp.dot(a, b, preferred_element_type=_F32)


def _dot_nt(a, b):
    return lax.dot_general(a, b, _NT, preferred_element_type=_F32)


def _for_head_group(w_ref, n_rows, n_heads, g, fn):
    w32 = w_ref.bitcast(jnp.uint32)
    npair = n_heads // 2
    grp = 4
    half = n_rows // 2
    span = n_rows * npair - (npair - grp)
    sub = w32.at[pl.ds(pl.multiple_of(g * grp, grp), span), :]
    for r in range(grp):
        ev = sub[pl.ds(r, half, stride=2 * npair), :]
        od = sub[pl.ds(r + npair, half, stride=2 * npair), :]
        lo = (ev & jnp.uint32(0xFFFF)) | (od << 16)
        hi = (ev >> 16) | (od & jnp.uint32(0xFFFF0000))
        h = 2 * (g * grp + r)
        fn(h, pltpu.bitcast(lo, _BF))
        fn(h + 1, pltpu.bitcast(hi, _BF))


@jax.jit
def pallas_gated_mix__compressed_kv_cla__sliding_block_cached__decode_kernel(
    A_x: jax.Array,
    A_c_kv: jax.Array,
    A_w_q: jax.Array,
    A_w_uk: jax.Array,
    A_w_uv: jax.Array,
    A_w_o: jax.Array,
    B_x: jax.Array,
    B_k_cache: jax.Array,
    B_v_cache: jax.Array,
    B_wq: jax.Array,
    B_wo: jax.Array,
    gate_w: jax.Array,
):
    del B_x
    B, Sq, M = A_x.shape
    Sk, Dc = A_c_kv.shape[1], A_c_kv.shape[2]
    H, D = A_w_q.shape[1], A_w_q.shape[2]
    Hq, Dh = 32, 128
    Hkv, SkB = B_k_cache.shape[1], B_k_cache.shape[2]
    W = min(4096, max(256, SkB // 4))
    rep = Hq // Hkv
    G = _G
    nck = Dc // 128
    CH = Sk // G
    QC = Hq * Dh // G
    scale_a = float(D) ** -0.5
    scale_b = float(Dh) ** -0.5
    assert Sq == 1 and B == 8 and D == 128 and Dh == 128 and rep == 4 and H == Hq == 8 * G
    assert Hkv == 2 * G and M == Dc == 4 * 128
    assert CH * Dc * 2 == _UNIT_BYTES and 4 * W * Dh * 2 == _UNIT_BYTES

    def kernel(x_hbm, c_hbm, wq_hbm, wuk_hbm, wuv_hbm, wo_hbm, k_hbm, v_hbm, bwq_hbm, bwo_hbm,
               gw_hbm, o_ref,
               x_s, gw_s, c_s, wq_s, wuk_s, wuv_s, wo_s, k_s, v_s, bwq_s, bwo_s,
               qb_s, qa_s, qabs_s, cabs_s, ctx_s, ob_s, obl_s, sems):

        def cp(src, dst, s):
            return pltpu.make_async_copy(src, dst, sems.at[s])

        def start_regions(regions, n_rows, s):
            rows = _DESC_BYTES // (2 * regions[0][0].shape[1])

            def body(i, carry):
                for r, (src, s0, dst, d0) in enumerate(regions):
                    cp(src.at[pl.ds(pl.multiple_of(s0 + i * rows, rows), rows), :],
                       dst.at[pl.ds(pl.multiple_of(d0 + i * rows, rows), rows), :],
                       s).start(priority=r % 2)
                return carry

            lax.fori_loop(0, n_rows // rows, body, 0)

        def start_rows(src, dst, row0, n_rows, s, n_regions):
            part = n_rows // n_regions
            start_regions([(src, row0 + r * part, dst, row0 + r * part) for r in range(n_regions)],
                          part, s)

        def wait_rows(src, dst, row0, n_rows, s):
            sl = pl.ds(row0, n_rows)
            cp(src.at[sl, :], dst.at[sl, :], s).wait()

        def unit_rows(ref):
            return _UNIT_BYTES // (2 * ref.shape[1])

        def start_unit(src, dst, u, s):
            start_rows(src, dst, u * unit_rows(src), unit_rows(src), s, _REGIONS)

        def wait_unit(src, dst, u, s):
            n = unit_rows(src)
            wait_rows(src, dst, pl.multiple_of(u * n, n), n, s)

        def start_bwq(g):
            rows = _DESC_BYTES // (2 * QC)
            cols = pl.ds(pl.multiple_of(g * QC, QC), QC)

            def body(i, carry):
                for r in range(2):
                    sl = pl.ds(pl.multiple_of(r * (M // 2) + i * rows, rows), rows)
                    cp(bwq_hbm.at[sl, cols], bwq_s.at[sl, cols], g).start(priority=r)
                return carry

            lax.fori_loop(0, M // 2 // rows, body, 0)

        def wait_bwq(g):
            cols = pl.ds(pl.multiple_of(g * QC, QC), QC)
            cp(bwq_hbm.at[:, cols], bwq_s.at[:, cols], g).wait()

        def start_kv(b, g):
            regions = []
            for src, dst in ((k_hbm, k_s), (v_hbm, v_s)):
                for t in range(2):
                    h = b * Hkv + 2 * g + t
                    for q in range(2):
                        regions.append((src, h * SkB + (SkB - W) + q * (W // 2),
                                        dst, h * W + q * (W // 2)))
            start_regions(regions, W // 2, g)

        def wait_kv(b, g):
            sl = pl.ds(pl.multiple_of((b * Hkv + 2 * g) * W, 2 * W), 2 * W)
            cp(k_hbm.at[pl.ds(0, 2 * W), :], k_s.at[sl, :], g).wait()
            cp(v_hbm.at[pl.ds(0, 2 * W), :], v_s.at[sl, :], g).wait()

        start_unit(wq_hbm, wq_s, 0, 0)
        cp(x_hbm, x_s, 0).start()
        cp(gw_hbm, gw_s, 0).start()
        for g in range(1, G):
            start_unit(wq_hbm, wq_s, g, g)
        cp(x_hbm, x_s, 0).wait()
        cp(gw_hbm, gw_s, 0).wait()

        def slot_wq(g, carry):
            wait_unit(wq_hbm, wq_s, g, g)
            start_unit(wuk_hbm, wuk_s, g, g)
            return carry

        lax.fori_loop(0, G, slot_wq, 0)

        x = x_s[...]
        gate = jax.nn.sigmoid(jnp.sum(
            x.astype(_F32) * gw_s[...].reshape(1, M).astype(_F32), axis=-1, keepdims=True))

        def qa_fn(h, w):
            qa_s[pl.ds(pl.multiple_of(h * B, B), B), :] = _dot(x, w)

        def slot_wuk(g, carry):
            wait_unit(wuk_hbm, wuk_s, g, g)
            start_bwq(g)
            _for_head_group(wq_s, M, H, g, qa_fn)
            return carry

        lax.fori_loop(0, G, slot_wuk, 0)

        def qabs_fn(h, w):
            rows = pl.ds(pl.multiple_of(h * B, B), B)
            r = _dot_nt(qa_s[rows, :].astype(_BF), w) * scale_a
            for k in range(nck):
                qabs_s[k, rows, :] = r[:, k * 128:(k + 1) * 128]

        def slot_bwq(g, carry):
            wait_bwq(g)
            start_unit(c_hbm, c_s, g, g)
            _for_head_group(wuk_s, Dc, H, g, qabs_fn)
            cols = pl.ds(pl.multiple_of(g * QC, QC), QC)
            q = _dot(x, bwq_s[:, cols]).astype(_BF).astype(_F32) * scale_b
            for r in range(8):
                qb_s[pl.ds(pl.multiple_of((g * 8 + r) * B, B), B), :] = q[:, r * Dh:(r + 1) * Dh]
            return carry

        lax.fori_loop(0, G, slot_bwq, 0)

        first = lax.broadcasted_iota(jnp.int32, (8, 1), 0) < rep

        def batch_body(b, carry):
            q = jnp.concatenate([qabs_s[k, pl.ds(b, H, stride=B), :] for k in range(nck)],
                                axis=1).astype(_BF)

            def slot_c(g, state):
                m_old, l_old, acc = state
                u = b * G + g
                wait_unit(c_hbm, c_s, u, g)
                start_kv(b, g)
                c = c_s.at[pl.ds(pl.multiple_of(u * CH, CH), CH), :]
                s = _dot_nt(q, c[...])
                m_new = jnp.maximum(m_old, jnp.max(s, axis=-1, keepdims=True))
                alpha = jnp.exp(m_old - m_new)
                p = jnp.exp(s - m_new)
                l_new = alpha * l_old + jnp.sum(p, axis=-1, keepdims=True)
                acc = alpha * acc + _dot(p.astype(_BF), c[...])
                return m_new, l_new, acc

            state0 = (jnp.full((H, 1), -jnp.inf, _F32), jnp.zeros((H, 1), _F32),
                      jnp.zeros((H, Dc), _F32))
            _, l, acc = lax.fori_loop(0, G, slot_c, state0)
            ctx = acc / l
            for k in range(nck):
                cabs_s[k, pl.ds(b, H, stride=B), :] = ctx[:, k * 128:(k + 1) * 128]

            def slot_kv(j, carry2):
                wait_kv(b, j)

                @pl.when(b < B - 1)
                def _():
                    start_unit(c_hbm, c_s, (b + 1) * G + j, j)

                @pl.when(b == B - 1)
                def _():
                    start_unit(wuv_hbm, wuv_s, j, j)

                rows8 = pl.ds(b + j * 8 * B, 8, stride=B)
                q8 = qb_s[rows8, :].astype(_BF)
                r0 = pl.ds(pl.multiple_of((b * Hkv + 2 * j) * W, W), W)
                r1 = pl.ds(pl.multiple_of((b * Hkv + 2 * j + 1) * W, W), W)
                sb = jnp.where(first, _dot_nt(q8, k_s[r0, :]), _dot_nt(q8, k_s[r1, :]))
                mb = jnp.max(sb, axis=-1, keepdims=True)
                pb = jnp.exp(sb - mb)
                lb = jnp.sum(pb, axis=-1, keepdims=True)
                pb = pb.astype(_BF)
                ob = jnp.where(first, _dot(pb, v_s[r0, :]), _dot(pb, v_s[r1, :]))
                ob_s[rows8, :] = ob / lb
                return carry2

            lax.fori_loop(0, G, slot_kv, 0)
            return carry

        lax.fori_loop(0, B, batch_body, 0)
        obl_s[...] = jnp.concatenate(
            [ob_s[h * B:(h + 1) * B, :] for h in range(Hq)], axis=1).astype(_BF)

        def slot_wuv(g, carry):
            wait_unit(wuv_hbm, wuv_s, g, g)
            start_unit(wo_hbm, wo_s, g, g)
            return carry

        lax.fori_loop(0, G, slot_wuv, 0)

        def ctx_fn(h, w):
            rows = pl.ds(pl.multiple_of(h * B, B), B)
            lhs = jnp.concatenate([cabs_s[k, rows, :] for k in range(nck)], axis=1)
            ctx_s[rows, :] = _dot(lhs.astype(_BF), w)

        def slot_wo(g, acc):
            wait_unit(wo_hbm, wo_s, g, g)

            @pl.when(g < G - 1)
            def _():
                start_rows(bwo_hbm, bwo_s, g * (8 * Dh), 8 * Dh, g, 2)

            @pl.when(g == G - 1)
            def _():
                start_rows(bwo_hbm, bwo_s, 24 * Dh, 4 * Dh, G - 1, 2)

            _for_head_group(wuv_s, Dc, H, g, ctx_fn)
            lhs = jnp.concatenate(
                [ctx_s[pl.ds(pl.multiple_of((g * 8 + r) * B, B), B), :] for r in range(8)],
                axis=1).astype(_BF)
            rows = pl.ds(pl.multiple_of(g * (8 * D), 8 * D), 8 * D)
            return acc + _dot(lhs, wo_s[rows, :])

        out_a = lax.fori_loop(0, G, slot_wo, jnp.zeros((B, M), _F32))

        def slot_bwo(g, acc):
            row0 = pl.multiple_of(g * (8 * Dh), 8 * Dh)
            wait_rows(bwo_hbm, bwo_s, row0, 8 * Dh, g)

            @pl.when(g < 2)
            def _():
                start_rows(bwo_hbm, bwo_s, (28 + 2 * g) * Dh, 2 * Dh, g, 2)

            rows = pl.ds(row0, 8 * Dh)
            return acc + _dot(obl_s[:, rows], bwo_s[rows, :])

        out_b = lax.fori_loop(0, 3, slot_bwo, jnp.zeros((B, M), _F32))
        for lo, hi, s in ((24, 28, 3), (28, 30, 0), (30, 32, 1)):
            wait_rows(bwo_hbm, bwo_s, lo * Dh, (hi - lo) * Dh, s)
            out_b = out_b + _dot(obl_s[:, lo * Dh:hi * Dh], bwo_s[lo * Dh:hi * Dh, :])

        out = gate * out_a + (1.0 - gate) * out_b
        o_ref[...] = out.astype(o_ref.dtype)

    any_spec = pl.BlockSpec(memory_space=pl.ANY)
    scratch = [
        pltpu.VMEM((B, M), _BF),
        pltpu.VMEM((M,), _BF),
        pltpu.VMEM((B * Sk, Dc), _BF),
        pltpu.VMEM((M * H, D), _BF),
        pltpu.VMEM((Dc * H, D), _BF),
        pltpu.VMEM((Dc * H, D), _BF),
        pltpu.VMEM((H * D, M), _BF),
        pltpu.VMEM((B * Hkv * W, Dh), _BF),
        pltpu.VMEM((B * Hkv * W, Dh), _BF),
        pltpu.VMEM((M, Hq * Dh), _BF),
        pltpu.VMEM((Hq * Dh, M), _BF),
        pltpu.VMEM((Hq * B, Dh), _F32),
        pltpu.VMEM((H * B, D), _F32),
        pltpu.VMEM((nck, H * B, 128), _F32),
        pltpu.VMEM((nck, H * B, 128), _F32),
        pltpu.VMEM((H * B, D), _F32),
        pltpu.VMEM((Hq * B, Dh), _F32),
        pltpu.VMEM((B, Hq * Dh), _BF),
        pltpu.SemaphoreType.DMA((G,)),
    ]
    out = pl.pallas_call(
        kernel,
        out_shape=jax.ShapeDtypeStruct((B, M), A_x.dtype),
        in_specs=[any_spec] * 11,
        out_specs=pl.BlockSpec(memory_space=pltpu.VMEM),
        scratch_shapes=scratch,
        compiler_params=pltpu.CompilerParams(vmem_limit_bytes=110 * 2**20),
    )(A_x.reshape(B, M), A_c_kv.reshape(B * Sk, Dc), A_w_q.reshape(M * H, D),
      A_w_uk.reshape(Dc * H, D), A_w_uv.reshape(Dc * H, D), A_w_o.reshape(H * D, M),
      B_k_cache.reshape(B * Hkv * SkB, Dh), B_v_cache.reshape(B * Hkv * SkB, Dh),
      B_wq, B_wo, gate_w)
    return out.reshape(B, Sq, M)
```

```python
import jax
import jax.numpy as jnp
from jax import lax
import jax.experimental.pallas as pl
import jax.experimental.pallas.tpu as pltpu

_BF = jnp.bfloat16
_F32 = jnp.float32
_NT = (((1,), (1,)), ((), ()))
_G = 4
_UNIT_BYTES = 1 << 20
_SPLIT_KIB = (48, 64, 16)
_ROTATE = 2


def _dot(a, b):
    return jnp.dot(a, b, preferred_element_type=_F32)


def _dot_nt(a, b):
    return lax.dot_general(a, b, _NT, preferred_element_type=_F32)


def _for_head_group(w_ref, n_rows, n_heads, g, fn):
    w32 = w_ref.bitcast(jnp.uint32)
    npair = n_heads // 2
    grp = 4
    half = n_rows // 2
    span = n_rows * npair - (npair - grp)
    sub = w32.at[pl.ds(pl.multiple_of(g * grp, grp), span), :]
    for r in range(grp):
        ev = sub[pl.ds(r, half, stride=2 * npair), :]
        od = sub[pl.ds(r + npair, half, stride=2 * npair), :]
        lo = (ev & jnp.uint32(0xFFFF)) | (od << 16)
        hi = (ev >> 16) | (od & jnp.uint32(0xFFFF0000))
        h = 2 * (g * grp + r)
        fn(h, pltpu.bitcast(lo, _BF))
        fn(h + 1, pltpu.bitcast(hi, _BF))


@jax.jit
def pallas_gated_mix__compressed_kv_cla__sliding_block_cached__decode_kernel(
    A_x: jax.Array,
    A_c_kv: jax.Array,
    A_w_q: jax.Array,
    A_w_uk: jax.Array,
    A_w_uv: jax.Array,
    A_w_o: jax.Array,
    B_x: jax.Array,
    B_k_cache: jax.Array,
    B_v_cache: jax.Array,
    B_wq: jax.Array,
    B_wo: jax.Array,
    gate_w: jax.Array,
):
    del B_x
    B, Sq, M = A_x.shape
    Sk, Dc = A_c_kv.shape[1], A_c_kv.shape[2]
    H, D = A_w_q.shape[1], A_w_q.shape[2]
    Hq, Dh = 32, 128
    Hkv, SkB = B_k_cache.shape[1], B_k_cache.shape[2]
    W = min(4096, max(256, SkB // 4))
    rep = Hq // Hkv
    G = _G
    nck = Dc // 128
    CH = Sk // G
    QC = Hq * Dh // G
    scale_a = float(D) ** -0.5
    scale_b = float(Dh) ** -0.5
    assert Sq == 1 and B == 8 and D == 128 and Dh == 128 and rep == 4 and H == Hq == 8 * G
    assert Hkv == 2 * G and M == Dc == 4 * 128
    assert CH * Dc * 2 == _UNIT_BYTES and 4 * W * Dh * 2 == _UNIT_BYTES

    def kernel(x_hbm, c_hbm, wq_hbm, wuk_hbm, wuv_hbm, wo_hbm, k_hbm, v_hbm, bwq_hbm, bwo_hbm,
               gw_hbm, o_ref,
               x_s, gw_s, c_s, wq_s, wuk_s, wuv_s, wo_s, k_s, v_s, bwq_s, bwo_s,
               qb_s, qa_s, qabs_s, cabs_s, ctx_s, ob_s, obl_s, sems):

        def cp(src, dst, s):
            return pltpu.make_async_copy(src, dst, sems.at[s])

        def start_regions(regions, n_rows, s, cols=None):
            row_bytes = 2 * (regions[0][0].shape[1] if cols is None else cols.size)
            rows = [kib * 1024 // row_bytes for kib in _SPLIT_KIB]
            rows = rows * (n_rows // sum(rows))
            assert sum(rows) == n_rows and all(r % 8 == 0 for r in rows)
            offs = [sum(rows[:i]) for i in range(len(rows))]
            cs = slice(None) if cols is None else cols
            for i in range(len(rows)):
                for r, (src, s0, dst, d0) in enumerate(regions):
                    k = (i + r * _ROTATE) % len(rows)
                    cp(src.at[pl.ds(pl.multiple_of(s0 + offs[k], 8), rows[k]), cs],
                       dst.at[pl.ds(pl.multiple_of(d0 + offs[k], 8), rows[k]), cs],
                       s).start(priority=r % 2)

        def start_rows(src, dst, row0, n_rows, s, n_regions):
            part = n_rows // n_regions
            start_regions([(src, row0 + r * part, dst, row0 + r * part) for r in range(n_regions)],
                          part, s)

        def wait_rows(src, dst, row0, n_rows, s):
            sl = pl.ds(row0, n_rows)
            cp(src.at[sl, :], dst.at[sl, :], s).wait()

        def unit_rows(ref):
            return _UNIT_BYTES // (2 * ref.shape[1])

        def start_unit(src, dst, u, s):
            start_rows(src, dst, u * unit_rows(src), unit_rows(src), s, 4)

        def wait_unit(src, dst, u, s):
            n = unit_rows(src)
            wait_rows(src, dst, pl.multiple_of(u * n, n), n, s)

        def start_bwq(g):
            cols = pl.ds(pl.multiple_of(g * QC, QC), QC)
            part = M // 8
            start_regions([(bwq_hbm, r * part, bwq_s, r * part) for r in range(8)], part, g, cols)

        def wait_bwq(g):
            cols = pl.ds(pl.multiple_of(g * QC, QC), QC)
            cp(bwq_hbm.at[:, cols], bwq_s.at[:, cols], g).wait()

        def start_kv(b, g):
            regions = []
            for src, dst in ((k_hbm, k_s), (v_hbm, v_s)):
                for t in range(2):
                    h = b * Hkv + 2 * g + t
                    for q in range(2):
                        regions.append((src, h * SkB + (SkB - W) + q * (W // 2),
                                        dst, h * W + q * (W // 2)))
            start_regions(regions, W // 2, g)

        def wait_kv(b, g):
            sl = pl.ds(pl.multiple_of((b * Hkv + 2 * g) * W, 2 * W), 2 * W)
            cp(k_hbm.at[pl.ds(0, 2 * W), :], k_s.at[sl, :], g).wait()
            cp(v_hbm.at[pl.ds(0, 2 * W), :], v_s.at[sl, :], g).wait()

        start_unit(wq_hbm, wq_s, 0, 0)
        cp(x_hbm, x_s, 0).start()
        cp(gw_hbm, gw_s, 0).start()
        for g in range(1, G):
            start_unit(wq_hbm, wq_s, g, g)
        cp(x_hbm, x_s, 0).wait()
        cp(gw_hbm, gw_s, 0).wait()

        def slot_wq(g, carry):
            wait_unit(wq_hbm, wq_s, g, g)
            start_unit(wuk_hbm, wuk_s, g, g)
            return carry

        lax.fori_loop(0, G, slot_wq, 0)

        x = x_s[...]
        gate = jax.nn.sigmoid(jnp.sum(
            x.astype(_F32) * gw_s[...].reshape(1, M).astype(_F32), axis=-1, keepdims=True))

        def qa_fn(h, w):
            qa_s[pl.ds(pl.multiple_of(h * B, B), B), :] = _dot(x, w)

        def slot_wuk(g, carry):
            wait_unit(wuk_hbm, wuk_s, g, g)
            start_bwq(g)
            _for_head_group(wq_s, M, H, g, qa_fn)
            return carry

        lax.fori_loop(0, G, slot_wuk, 0)

        def qabs_fn(h, w):
            rows = pl.ds(pl.multiple_of(h * B, B), B)
            r = _dot_nt(qa_s[rows, :].astype(_BF), w) * scale_a
            for k in range(nck):
                qabs_s[k, rows, :] = r[:, k * 128:(k + 1) * 128]

        def slot_bwq(g, carry):
            wait_bwq(g)
            start_unit(c_hbm, c_s, g, g)
            _for_head_group(wuk_s, Dc, H, g, qabs_fn)
            cols = pl.ds(pl.multiple_of(g * QC, QC), QC)
            q = _dot(x, bwq_s[:, cols]).astype(_BF).astype(_F32) * scale_b
            for r in range(8):
                qb_s[pl.ds(pl.multiple_of((g * 8 + r) * B, B), B), :] = q[:, r * Dh:(r + 1) * Dh]
            return carry

        lax.fori_loop(0, G, slot_bwq, 0)

        first = lax.broadcasted_iota(jnp.int32, (8, 1), 0) < rep

        def batch_body(b, carry):
            q = jnp.concatenate([qabs_s[k, pl.ds(b, H, stride=B), :] for k in range(nck)],
                                axis=1).astype(_BF)

            def slot_c(g, state):
                m_old, l_old, acc = state
                u = b * G + g
                wait_unit(c_hbm, c_s, u, g)
                start_kv(b, g)
                c = c_s.at[pl.ds(pl.multiple_of(u * CH, CH), CH), :]
                s = _dot_nt(q, c[...])
                m_new = jnp.maximum(m_old, jnp.max(s, axis=-1, keepdims=True))
                alpha = jnp.exp(m_old - m_new)
                p = jnp.exp(s - m_new)
                l_new = alpha * l_old + jnp.sum(p, axis=-1, keepdims=True)
                acc = alpha * acc + _dot(p.astype(_BF), c[...])
                return m_new, l_new, acc

            state0 = (jnp.full((H, 1), -jnp.inf, _F32), jnp.zeros((H, 1), _F32),
                      jnp.zeros((H, Dc), _F32))
            _, l, acc = lax.fori_loop(0, G, slot_c, state0)
            ctx = acc / l
            for k in range(nck):
                cabs_s[k, pl.ds(b, H, stride=B), :] = ctx[:, k * 128:(k + 1) * 128]

            def slot_kv(j, carry2):
                wait_kv(b, j)

                @pl.when(b < B - 1)
                def _():
                    start_unit(c_hbm, c_s, (b + 1) * G + j, j)

                @pl.when(b == B - 1)
                def _():
                    start_unit(wuv_hbm, wuv_s, j, j)

                rows8 = pl.ds(b + j * 8 * B, 8, stride=B)
                q8 = qb_s[rows8, :].astype(_BF)
                r0 = pl.ds(pl.multiple_of((b * Hkv + 2 * j) * W, W), W)
                r1 = pl.ds(pl.multiple_of((b * Hkv + 2 * j + 1) * W, W), W)
                sb = jnp.where(first, _dot_nt(q8, k_s[r0, :]), _dot_nt(q8, k_s[r1, :]))
                mb = jnp.max(sb, axis=-1, keepdims=True)
                pb = jnp.exp(sb - mb)
                lb = jnp.sum(pb, axis=-1, keepdims=True)
                pb = pb.astype(_BF)
                ob = jnp.where(first, _dot(pb, v_s[r0, :]), _dot(pb, v_s[r1, :]))
                ob_s[rows8, :] = ob / lb
                return carry2

            lax.fori_loop(0, G, slot_kv, 0)
            return carry

        lax.fori_loop(0, B, batch_body, 0)
        obl_s[...] = jnp.concatenate(
            [ob_s[h * B:(h + 1) * B, :] for h in range(Hq)], axis=1).astype(_BF)

        def slot_wuv(g, carry):
            wait_unit(wuv_hbm, wuv_s, g, g)
            start_unit(wo_hbm, wo_s, g, g)
            return carry

        lax.fori_loop(0, G, slot_wuv, 0)

        def ctx_fn(h, w):
            rows = pl.ds(pl.multiple_of(h * B, B), B)
            lhs = jnp.concatenate([cabs_s[k, rows, :] for k in range(nck)], axis=1)
            ctx_s[rows, :] = _dot(lhs.astype(_BF), w)

        def slot_wo(g, acc):
            wait_unit(wo_hbm, wo_s, g, g)

            @pl.when(g < G - 1)
            def _():
                start_rows(bwo_hbm, bwo_s, g * (8 * Dh), 8 * Dh, g, 4)

            @pl.when(g == G - 1)
            def _():
                start_rows(bwo_hbm, bwo_s, 24 * Dh, 4 * Dh, G - 1, 4)

            _for_head_group(wuv_s, Dc, H, g, ctx_fn)
            lhs = jnp.concatenate(
                [ctx_s[pl.ds(pl.multiple_of((g * 8 + r) * B, B), B), :] for r in range(8)],
                axis=1).astype(_BF)
            rows = pl.ds(pl.multiple_of(g * (8 * D), 8 * D), 8 * D)
            return acc + _dot(lhs, wo_s[rows, :])

        out_a = lax.fori_loop(0, G, slot_wo, jnp.zeros((B, M), _F32))

        def slot_bwo(g, acc):
            row0 = pl.multiple_of(g * (8 * Dh), 8 * Dh)
            wait_rows(bwo_hbm, bwo_s, row0, 8 * Dh, g)

            @pl.when(g < 2)
            def _():
                start_rows(bwo_hbm, bwo_s, (28 + 2 * g) * Dh, 2 * Dh, g, 2)

            rows = pl.ds(row0, 8 * Dh)
            return acc + _dot(obl_s[:, rows], bwo_s[rows, :])

        out_b = lax.fori_loop(0, 3, slot_bwo, jnp.zeros((B, M), _F32))
        for lo, hi, s in ((24, 28, 3), (28, 30, 0), (30, 32, 1)):
            wait_rows(bwo_hbm, bwo_s, lo * Dh, (hi - lo) * Dh, s)
            out_b = out_b + _dot(obl_s[:, lo * Dh:hi * Dh], bwo_s[lo * Dh:hi * Dh, :])

        out = gate * out_a + (1.0 - gate) * out_b
        o_ref[...] = out.astype(o_ref.dtype)

    any_spec = pl.BlockSpec(memory_space=pl.ANY)
    scratch = [
        pltpu.VMEM((B, M), _BF),
        pltpu.VMEM((M,), _BF),
        pltpu.VMEM((B * Sk, Dc), _BF),
        pltpu.VMEM((M * H, D), _BF),
        pltpu.VMEM((Dc * H, D), _BF),
        pltpu.VMEM((Dc * H, D), _BF),
        pltpu.VMEM((H * D, M), _BF),
        pltpu.VMEM((B * Hkv * W, Dh), _BF),
        pltpu.VMEM((B * Hkv * W, Dh), _BF),
        pltpu.VMEM((M, Hq * Dh), _BF),
        pltpu.VMEM((Hq * Dh, M), _BF),
        pltpu.VMEM((Hq * B, Dh), _F32),
        pltpu.VMEM((H * B, D), _F32),
        pltpu.VMEM((nck, H * B, 128), _F32),
        pltpu.VMEM((nck, H * B, 128), _F32),
        pltpu.VMEM((H * B, D), _F32),
        pltpu.VMEM((Hq * B, Dh), _F32),
        pltpu.VMEM((B, Hq * Dh), _BF),
        pltpu.SemaphoreType.DMA((G,)),
    ]
    out = pl.pallas_call(
        kernel,
        out_shape=jax.ShapeDtypeStruct((B, M), A_x.dtype),
        in_specs=[any_spec] * 11,
        out_specs=pl.BlockSpec(memory_space=pltpu.VMEM),
        scratch_shapes=scratch,
        compiler_params=pltpu.CompilerParams(vmem_limit_bytes=110 * 2**20),
    )(A_x.reshape(B, M), A_c_kv.reshape(B * Sk, Dc), A_w_q.reshape(M * H, D),
      A_w_uk.reshape(Dc * H, D), A_w_uv.reshape(Dc * H, D), A_w_o.reshape(H * D, M),
      B_k_cache.reshape(B * Hkv * SkB, Dh), B_v_cache.reshape(B * Hkv * SkB, Dh),
      B_wq, B_wo, gate_w)
    return out.reshape(B, Sq, M)
```

```python
import jax
import jax.numpy as jnp
from jax import lax
import jax.experimental.pallas as pl
import jax.experimental.pallas.tpu as pltpu

_BF = jnp.bfloat16
_F32 = jnp.float32
_NT = (((1,), (1,)), ((), ()))
_G = 4
_UNIT_BYTES = 1 << 20
_SPLIT_A = ((48, 64, 16), 2)
_SPLIT_B = ((48, 56, 24), 0)


def _dot(a, b):
    return jnp.dot(a, b, preferred_element_type=_F32)


def _dot_nt(a, b):
    return lax.dot_general(a, b, _NT, preferred_element_type=_F32)


def _for_head_group(w_ref, n_rows, n_heads, g, fn):
    w32 = w_ref.bitcast(jnp.uint32)
    npair = n_heads // 2
    grp = 4
    half = n_rows // 2
    span = n_rows * npair - (npair - grp)
    sub = w32.at[pl.ds(pl.multiple_of(g * grp, grp), span), :]
    for r in range(grp):
        ev = sub[pl.ds(r, half, stride=2 * npair), :]
        od = sub[pl.ds(r + npair, half, stride=2 * npair), :]
        lo = (ev & jnp.uint32(0xFFFF)) | (od << 16)
        hi = (ev >> 16) | (od & jnp.uint32(0xFFFF0000))
        h = 2 * (g * grp + r)
        fn(h, pltpu.bitcast(lo, _BF))
        fn(h + 1, pltpu.bitcast(hi, _BF))


@jax.jit
def pallas_gated_mix__compressed_kv_cla__sliding_block_cached__decode_kernel(
    A_x: jax.Array,
    A_c_kv: jax.Array,
    A_w_q: jax.Array,
    A_w_uk: jax.Array,
    A_w_uv: jax.Array,
    A_w_o: jax.Array,
    B_x: jax.Array,
    B_k_cache: jax.Array,
    B_v_cache: jax.Array,
    B_wq: jax.Array,
    B_wo: jax.Array,
    gate_w: jax.Array,
):
    del B_x
    B, Sq, M = A_x.shape
    Sk, Dc = A_c_kv.shape[1], A_c_kv.shape[2]
    H, D = A_w_q.shape[1], A_w_q.shape[2]
    Hq, Dh = 32, 128
    Hkv, SkB = B_k_cache.shape[1], B_k_cache.shape[2]
    W = min(4096, max(256, SkB // 4))
    rep = Hq // Hkv
    G = _G
    nck = Dc // 128
    CH = Sk // G
    PC = CH // G
    QC = Hq * Dh // G
    scale_a = float(D) ** -0.5
    scale_b = float(Dh) ** -0.5
    assert Sq == 1 and B == 8 and D == 128 and Dh == 128 and rep == 4 and H == Hq == 8 * G
    assert Hkv == 2 * G and M == Dc == 4 * 128
    assert CH * Dc * 2 == _UNIT_BYTES and 4 * W * Dh * 2 == _UNIT_BYTES

    def kernel(x_hbm, c_hbm, wq_hbm, wuk_hbm, wuv_hbm, wo_hbm, k_hbm, v_hbm, bwq_hbm, bwo_hbm,
               gw_hbm, o_ref,
               x_s, gw_s, c_s, wq_s, wuk_s, wuv_s, wo_s, k_s, v_s, bwq_s, bwo_s,
               qb_s, qa_s, qabs_s, cabs_s, ctx_s, ob_s, obl_s, sems):

        def cp(src, dst, s):
            return pltpu.make_async_copy(src, dst, sems.at[s])

        def start_regions(regions, n_rows, s, split, cols=None):
            row_bytes = 2 * (regions[0][0].shape[1] if cols is None else cols.size)
            sizes, rotate = split
            rows = [kib * 1024 // row_bytes for kib in sizes]
            rows = rows * (n_rows // sum(rows))
            assert sum(rows) == n_rows and all(r % 8 == 0 for r in rows)
            offs = [sum(rows[:i]) for i in range(len(rows))]
            cs = slice(None) if cols is None else cols
            for i in range(len(rows)):
                for r, (src, s0, dst, d0) in enumerate(regions):
                    k = (i + r * rotate) % len(rows)
                    cp(src.at[pl.ds(pl.multiple_of(s0 + offs[k], 8), rows[k]), cs],
                       dst.at[pl.ds(pl.multiple_of(d0 + offs[k], 8), rows[k]), cs],
                       s).start(priority=r % 2)

        def start_rows(src, dst, row0, n_rows, s, n_regions):
            part = n_rows // n_regions
            start_regions([(src, row0 + r * part, dst, row0 + r * part) for r in range(n_regions)],
                          part, s, _SPLIT_A)

        def wait_rows(src, dst, row0, n_rows, s):
            sl = pl.ds(row0, n_rows)
            cp(src.at[sl, :], dst.at[sl, :], s).wait()

        def unit_rows(ref):
            return _UNIT_BYTES // (2 * ref.shape[1])

        def start_unit(src, dst, u, s):
            start_rows(src, dst, u * unit_rows(src), unit_rows(src), s, 4)

        def start_spread(src, dst, a, g):
            n = unit_rows(src)
            regions = [a * G * n + j * n + g * (n // G) + q * (n // G // 2)
                       for j in range(G) for q in range(2)]
            start_regions([(src, r, dst, r) for r in regions], n // G // 2, g, _SPLIT_B)

        def wait_unit(src, dst, u, s):
            n = unit_rows(src)
            wait_rows(src, dst, pl.multiple_of(u * n, n), n, s)

        def wait_spread(src, dst, a, g):
            n = unit_rows(src)
            for j in range(G):
                wait_rows(src, dst, pl.multiple_of((a * G + j) * n + g * (n // G), n // G), n // G, g)

        def start_bwq(g):
            cols = pl.ds(pl.multiple_of(g * QC, QC), QC)
            part = M // 8
            start_regions([(bwq_hbm, r * part, bwq_s, r * part) for r in range(8)], part, g,
                          _SPLIT_A, cols)

        def wait_bwq(g):
            cols = pl.ds(pl.multiple_of(g * QC, QC), QC)
            cp(bwq_hbm.at[:, cols], bwq_s.at[:, cols], g).wait()

        def start_kv(b, g):
            regions = []
            for src, dst in ((k_hbm, k_s), (v_hbm, v_s)):
                for t in range(2):
                    h = b * Hkv + 2 * g + t
                    for q in range(2):
                        regions.append((src, h * SkB + (SkB - W) + q * (W // 2),
                                        dst, h * W + q * (W // 2)))
            start_regions(regions, W // 2, g, _SPLIT_A)

        def wait_kv(b, g):
            for src, dst in ((k_hbm, k_s), (v_hbm, v_s)):
                for t in range(2):
                    h = b * Hkv + 2 * g + t
                    cp(src.at[pl.ds(pl.multiple_of(h * SkB + (SkB - W), W), W), :],
                       dst.at[pl.ds(pl.multiple_of(h * W, W), W), :], g).wait()

        start_spread(wq_hbm, wq_s, 0, 0)
        cp(x_hbm, x_s, 0).start()
        cp(gw_hbm, gw_s, 0).start()
        for g in range(1, G):
            start_spread(wq_hbm, wq_s, 0, g)
        cp(x_hbm, x_s, 0).wait()
        cp(gw_hbm, gw_s, 0).wait()

        def slot_wq(g, carry):
            wait_spread(wq_hbm, wq_s, 0, g)
            start_spread(wuk_hbm, wuk_s, 0, g)
            return carry

        lax.fori_loop(0, G, slot_wq, 0)

        x = x_s[...]
        gate = jax.nn.sigmoid(jnp.sum(
            x.astype(_F32) * gw_s[...].reshape(1, M).astype(_F32), axis=-1, keepdims=True))

        def qa_fn(h, w):
            qa_s[pl.ds(pl.multiple_of(h * B, B), B), :] = _dot(x, w)

        def slot_wuk(g, carry):
            wait_spread(wuk_hbm, wuk_s, 0, g)
            start_bwq(g)
            _for_head_group(wq_s, M, H, g, qa_fn)
            return carry

        lax.fori_loop(0, G, slot_wuk, 0)

        def qabs_fn(h, w):
            rows = pl.ds(pl.multiple_of(h * B, B), B)
            r = _dot_nt(qa_s[rows, :].astype(_BF), w) * scale_a
            for k in range(nck):
                qabs_s[k, rows, :] = r[:, k * 128:(k + 1) * 128]

        def slot_bwq(g, carry):
            wait_bwq(g)
            start_spread(c_hbm, c_s, 0, g)
            _for_head_group(wuk_s, Dc, H, g, qabs_fn)
            cols = pl.ds(pl.multiple_of(g * QC, QC), QC)
            q = _dot(x, bwq_s[:, cols]).astype(_BF).astype(_F32) * scale_b
            for r in range(8):
                qb_s[pl.ds(pl.multiple_of((g * 8 + r) * B, B), B), :] = q[:, r * Dh:(r + 1) * Dh]
            return carry

        lax.fori_loop(0, G, slot_bwq, 0)

        first = lax.broadcasted_iota(jnp.int32, (8, 1), 0) < rep

        def batch_body(b, carry):
            q = jnp.concatenate([qabs_s[k, pl.ds(b, H, stride=B), :] for k in range(nck)],
                                axis=1).astype(_BF)

            def slot_c(g, state):
                m_old, l_old, acc = state
                wait_spread(c_hbm, c_s, b, g)
                start_kv(b, g)
                pieces = [c_s.at[pl.ds(pl.multiple_of((b * G + j) * CH + g * PC, PC), PC), :]
                          for j in range(G)]
                s = jnp.concatenate([_dot_nt(q, c[...]) for c in pieces], axis=1)
                m_new = jnp.maximum(m_old, jnp.max(s, axis=-1, keepdims=True))
                alpha = jnp.exp(m_old - m_new)
                p = jnp.exp(s - m_new)
                l_new = alpha * l_old + jnp.sum(p, axis=-1, keepdims=True)
                p = p.astype(_BF)
                pv = _dot(p[:, :PC], pieces[0][...])
                for j in range(1, G):
                    pv = pv + _dot(p[:, j * PC:(j + 1) * PC], pieces[j][...])
                acc = alpha * acc + pv
                return m_new, l_new, acc

            state0 = (jnp.full((H, 1), -jnp.inf, _F32), jnp.zeros((H, 1), _F32),
                      jnp.zeros((H, Dc), _F32))
            _, l, acc = lax.fori_loop(0, G, slot_c, state0)
            ctx = acc / l
            for k in range(nck):
                cabs_s[k, pl.ds(b, H, stride=B), :] = ctx[:, k * 128:(k + 1) * 128]

            def slot_kv(j, carry2):
                wait_kv(b, j)

                @pl.when(b < B - 1)
                def _():
                    start_spread(c_hbm, c_s, b + 1, j)

                @pl.when(b == B - 1)
                def _():
                    start_spread(wuv_hbm, wuv_s, 0, j)

                rows8 = pl.ds(b + j * 8 * B, 8, stride=B)
                q8 = qb_s[rows8, :].astype(_BF)
                r0 = pl.ds(pl.multiple_of((b * Hkv + 2 * j) * W, W), W)
                r1 = pl.ds(pl.multiple_of((b * Hkv + 2 * j + 1) * W, W), W)
                sb = jnp.where(first, _dot_nt(q8, k_s[r0, :]), _dot_nt(q8, k_s[r1, :]))
                mb = jnp.max(sb, axis=-1, keepdims=True)
                pb = jnp.exp(sb - mb)
                lb = jnp.sum(pb, axis=-1, keepdims=True)
                pb = pb.astype(_BF)
                ob = jnp.where(first, _dot(pb, v_s[r0, :]), _dot(pb, v_s[r1, :]))
                ob_s[rows8, :] = ob / lb
                return carry2

            lax.fori_loop(0, G, slot_kv, 0)
            return carry

        lax.fori_loop(0, B, batch_body, 0)
        obl_s[...] = jnp.concatenate(
            [ob_s[h * B:(h + 1) * B, :] for h in range(Hq)], axis=1).astype(_BF)

        def slot_wuv(g, carry):
            wait_spread(wuv_hbm, wuv_s, 0, g)
            start_unit(wo_hbm, wo_s, g, g)
            return carry

        lax.fori_loop(0, G, slot_wuv, 0)

        def ctx_fn(h, w):
            rows = pl.ds(pl.multiple_of(h * B, B), B)
            lhs = jnp.concatenate([cabs_s[k, rows, :] for k in range(nck)], axis=1)
            ctx_s[rows, :] = _dot(lhs.astype(_BF), w)

        def slot_wo(g, acc):
            wait_unit(wo_hbm, wo_s, g, g)

            @pl.when(g < G - 1)
            def _():
                start_rows(bwo_hbm, bwo_s, g * (8 * Dh), 8 * Dh, g, 4)

            @pl.when(g == G - 1)
            def _():
                start_rows(bwo_hbm, bwo_s, 24 * Dh, 4 * Dh, G - 1, 4)

            _for_head_group(wuv_s, Dc, H, g, ctx_fn)
            lhs = jnp.concatenate(
                [ctx_s[pl.ds(pl.multiple_of((g * 8 + r) * B, B), B), :] for r in range(8)],
                axis=1).astype(_BF)
            rows = pl.ds(pl.multiple_of(g * (8 * D), 8 * D), 8 * D)
            return acc + _dot(lhs, wo_s[rows, :])

        out_a = lax.fori_loop(0, G, slot_wo, jnp.zeros((B, M), _F32))

        def slot_bwo(g, acc):
            row0 = pl.multiple_of(g * (8 * Dh), 8 * Dh)
            wait_rows(bwo_hbm, bwo_s, row0, 8 * Dh, g)

            @pl.when(g < 2)
            def _():
                start_rows(bwo_hbm, bwo_s, (28 + 2 * g) * Dh, 2 * Dh, g, 2)

            rows = pl.ds(row0, 8 * Dh)
            return acc + _dot(obl_s[:, rows], bwo_s[rows, :])

        out_b = lax.fori_loop(0, 3, slot_bwo, jnp.zeros((B, M), _F32))
        for lo, hi, s in ((24, 28, 3), (28, 30, 0), (30, 32, 1)):
            wait_rows(bwo_hbm, bwo_s, lo * Dh, (hi - lo) * Dh, s)
            out_b = out_b + _dot(obl_s[:, lo * Dh:hi * Dh], bwo_s[lo * Dh:hi * Dh, :])

        out = gate * out_a + (1.0 - gate) * out_b
        o_ref[...] = out.astype(o_ref.dtype)

    any_spec = pl.BlockSpec(memory_space=pl.ANY)
    scratch = [
        pltpu.VMEM((B, M), _BF),
        pltpu.VMEM((M,), _BF),
        pltpu.VMEM((B * Sk, Dc), _BF),
        pltpu.VMEM((M * H, D), _BF),
        pltpu.VMEM((Dc * H, D), _BF),
        pltpu.VMEM((Dc * H, D), _BF),
        pltpu.VMEM((H * D, M), _BF),
        pltpu.VMEM((B * Hkv * W, Dh), _BF),
        pltpu.VMEM((B * Hkv * W, Dh), _BF),
        pltpu.VMEM((M, Hq * Dh), _BF),
        pltpu.VMEM((Hq * Dh, M), _BF),
        pltpu.VMEM((Hq * B, Dh), _F32),
        pltpu.VMEM((H * B, D), _F32),
        pltpu.VMEM((nck, H * B, 128), _F32),
        pltpu.VMEM((nck, H * B, 128), _F32),
        pltpu.VMEM((H * B, D), _F32),
        pltpu.VMEM((Hq * B, Dh), _F32),
        pltpu.VMEM((B, Hq * Dh), _BF),
        pltpu.SemaphoreType.DMA((G,)),
    ]
    out = pl.pallas_call(
        kernel,
        out_shape=jax.ShapeDtypeStruct((B, M), A_x.dtype),
        in_specs=[any_spec] * 11,
        out_specs=pl.BlockSpec(memory_space=pltpu.VMEM),
        scratch_shapes=scratch,
        compiler_params=pltpu.CompilerParams(vmem_limit_bytes=110 * 2**20),
    )(A_x.reshape(B, M), A_c_kv.reshape(B * Sk, Dc), A_w_q.reshape(M * H, D),
      A_w_uk.reshape(Dc * H, D), A_w_uv.reshape(Dc * H, D), A_w_o.reshape(H * D, M),
      B_k_cache.reshape(B * Hkv * SkB, Dh), B_v_cache.reshape(B * Hkv * SkB, Dh),
      B_wq, B_wo, gate_w)
    return out.reshape(B, Sq, M)
```

```python
import jax
import jax.numpy as jnp
from jax import lax
import jax.experimental.pallas as pl
import jax.experimental.pallas.tpu as pltpu

_BF = jnp.bfloat16
_F32 = jnp.float32
_NT = (((1,), (1,)), ((), ()))
_G = 4
_UNIT_BYTES = 1 << 20
_SPLIT_KIB = (48, 48, 32)


def _dot(a, b):
    return jnp.dot(a, b, preferred_element_type=_F32)


def _dot_nt(a, b):
    return lax.dot_general(a, b, _NT, preferred_element_type=_F32)


def _for_head_group(w_ref, n_rows, n_heads, g, fn):
    w32 = w_ref.bitcast(jnp.uint32)
    npair = n_heads // 2
    grp = 4
    half = n_rows // 2
    span = n_rows * npair - (npair - grp)
    sub = w32.at[pl.ds(pl.multiple_of(g * grp, grp), span), :]
    for r in range(grp):
        ev = sub[pl.ds(r, half, stride=2 * npair), :]
        od = sub[pl.ds(r + npair, half, stride=2 * npair), :]
        lo = (ev & jnp.uint32(0xFFFF)) | (od << 16)
        hi = (ev >> 16) | (od & jnp.uint32(0xFFFF0000))
        h = 2 * (g * grp + r)
        fn(h, pltpu.bitcast(lo, _BF))
        fn(h + 1, pltpu.bitcast(hi, _BF))


@jax.jit
def pallas_gated_mix__compressed_kv_cla__sliding_block_cached__decode_kernel(
    A_x: jax.Array,
    A_c_kv: jax.Array,
    A_w_q: jax.Array,
    A_w_uk: jax.Array,
    A_w_uv: jax.Array,
    A_w_o: jax.Array,
    B_x: jax.Array,
    B_k_cache: jax.Array,
    B_v_cache: jax.Array,
    B_wq: jax.Array,
    B_wo: jax.Array,
    gate_w: jax.Array,
):
    del B_x
    B, Sq, M = A_x.shape
    Sk, Dc = A_c_kv.shape[1], A_c_kv.shape[2]
    H, D = A_w_q.shape[1], A_w_q.shape[2]
    Hq, Dh = 32, 128
    Hkv, SkB = B_k_cache.shape[1], B_k_cache.shape[2]
    W = min(4096, max(256, SkB // 4))
    rep = Hq // Hkv
    G = _G
    nck = Dc // 128
    CH = Sk // G
    PC = CH // G
    QC = Hq * Dh // G
    scale_a = float(D) ** -0.5
    scale_b = float(Dh) ** -0.5
    assert Sq == 1 and B == 8 and D == 128 and Dh == 128 and rep == 4 and H == Hq == 8 * G
    assert Hkv == 2 * G and M == Dc == 4 * 128
    assert CH * Dc * 2 == _UNIT_BYTES and 4 * W * Dh * 2 == _UNIT_BYTES

    def kernel(x_hbm, c_hbm, wq_hbm, wuk_hbm, wuv_hbm, wo_hbm, k_hbm, v_hbm, bwq_hbm, bwo_hbm,
               gw_hbm, o_ref,
               x_s, gw_s, c_s, wq_s, wuk_s, wuv_s, wo_s, k_s, v_s, bwq_s, bwo_s,
               qb_s, qa_s, qabs_s, cabs_s, ctx_s, ob_s, obl_s, sems):

        def cp(src, dst, s):
            return pltpu.make_async_copy(src, dst, sems.at[s])

        def start_regions(regions, n_rows, s, cols=None):
            row_bytes = 2 * (regions[0][0].shape[1] if cols is None else cols.size)
            rows = [kib * 1024 // row_bytes for kib in _SPLIT_KIB]
            rows = rows * (n_rows // sum(rows))
            assert sum(rows) == n_rows and all(r % 8 == 0 for r in rows)
            cs = slice(None) if cols is None else cols
            off = 0
            for n in rows:
                for r, (src, s0, dst, d0) in enumerate(regions):
                    cp(src.at[pl.ds(pl.multiple_of(s0 + off, 8), n), cs],
                       dst.at[pl.ds(pl.multiple_of(d0 + off, 8), n), cs],
                       s).start(priority=r % 2)
                off += n

        def start_rows(src, dst, row0, n_rows, s, n_regions):
            part = n_rows // n_regions
            start_regions([(src, row0 + r * part, dst, row0 + r * part) for r in range(n_regions)],
                          part, s)

        def wait_rows(src, dst, row0, n_rows, s):
            sl = pl.ds(row0, n_rows)
            cp(src.at[sl, :], dst.at[sl, :], s).wait()

        def unit_rows(ref):
            return _UNIT_BYTES // (2 * ref.shape[1])

        def start_unit(src, dst, u, s):
            start_rows(src, dst, u * unit_rows(src), unit_rows(src), s, 4)

        def start_spread(src, dst, a, g):
            n = unit_rows(src)
            regions = [a * G * n + j * n + g * (n // G) + q * (n // G // 2)
                       for j in range(G) for q in range(2)]
            start_regions([(src, r, dst, r) for r in regions], n // G // 2, g)

        def wait_unit(src, dst, u, s):
            n = unit_rows(src)
            wait_rows(src, dst, pl.multiple_of(u * n, n), n, s)

        def wait_spread(src, dst, a, g):
            n = unit_rows(src)
            for j in range(G):
                wait_rows(src, dst, pl.multiple_of((a * G + j) * n + g * (n // G), n // G), n // G, g)

        def start_bwq(g):
            cols = pl.ds(pl.multiple_of(g * QC, QC), QC)
            part = M // 8
            start_regions([(bwq_hbm, r * part, bwq_s, r * part) for r in range(8)], part, g, cols)

        def wait_bwq(g):
            cols = pl.ds(pl.multiple_of(g * QC, QC), QC)
            cp(bwq_hbm.at[:, cols], bwq_s.at[:, cols], g).wait()

        def start_kv(b, g):
            regions = []
            for src, dst in ((k_hbm, k_s), (v_hbm, v_s)):
                for t in range(2):
                    h = b * Hkv + 2 * g + t
                    for q in range(2):
                        regions.append((src, h * SkB + (SkB - W) + q * (W // 2),
                                        dst, h * W + q * (W // 2)))
            start_regions(regions, W // 2, g)

        def wait_kv(b, g):
            for src, dst in ((k_hbm, k_s), (v_hbm, v_s)):
                for t in range(2):
                    h = b * Hkv + 2 * g + t
                    cp(src.at[pl.ds(pl.multiple_of(h * SkB + (SkB - W), W), W), :],
                       dst.at[pl.ds(pl.multiple_of(h * W, W), W), :], g).wait()

        start_spread(wq_hbm, wq_s, 0, 0)
        cp(x_hbm, x_s, 0).start()
        cp(gw_hbm, gw_s, 0).start()
        for g in range(1, G):
            start_spread(wq_hbm, wq_s, 0, g)
        cp(x_hbm, x_s, 0).wait()
        cp(gw_hbm, gw_s, 0).wait()

        def slot_wq(g, carry):
            wait_spread(wq_hbm, wq_s, 0, g)
            start_spread(wuk_hbm, wuk_s, 0, g)
            return carry

        lax.fori_loop(0, G, slot_wq, 0)

        x = x_s[...]
        gate = jax.nn.sigmoid(jnp.sum(
            x.astype(_F32) * gw_s[...].reshape(1, M).astype(_F32), axis=-1, keepdims=True))

        def qa_fn(h, w):
            qa_s[pl.ds(pl.multiple_of(h * B, B), B), :] = _dot(x, w)

        def slot_wuk(g, carry):
            wait_spread(wuk_hbm, wuk_s, 0, g)
            start_bwq(g)
            _for_head_group(wq_s, M, H, g, qa_fn)
            return carry

        lax.fori_loop(0, G, slot_wuk, 0)

        def qabs_fn(h, w):
            rows = pl.ds(pl.multiple_of(h * B, B), B)
            r = _dot_nt(qa_s[rows, :].astype(_BF), w) * scale_a
            for k in range(nck):
                qabs_s[k, rows, :] = r[:, k * 128:(k + 1) * 128]

        def slot_bwq(g, carry):
            wait_bwq(g)
            start_spread(c_hbm, c_s, 0, g)
            _for_head_group(wuk_s, Dc, H, g, qabs_fn)
            cols = pl.ds(pl.multiple_of(g * QC, QC), QC)
            q = _dot(x, bwq_s[:, cols]).astype(_BF).astype(_F32) * scale_b
            for r in range(8):
                qb_s[pl.ds(pl.multiple_of((g * 8 + r) * B, B), B), :] = q[:, r * Dh:(r + 1) * Dh]
            return carry

        lax.fori_loop(0, G, slot_bwq, 0)

        first = lax.broadcasted_iota(jnp.int32, (8, 1), 0) < rep

        def batch_body(b, carry):
            q = jnp.concatenate([qabs_s[k, pl.ds(b, H, stride=B), :] for k in range(nck)],
                                axis=1).astype(_BF)

            def slot_c(g, state):
                m_old, l_old, acc = state
                wait_spread(c_hbm, c_s, b, g)
                start_kv(b, g)
                pieces = [c_s.at[pl.ds(pl.multiple_of((b * G + j) * CH + g * PC, PC), PC), :]
                          for j in range(G)]
                s = jnp.concatenate([_dot_nt(q, c[...]) for c in pieces], axis=1)
                m_new = jnp.maximum(m_old, jnp.max(s, axis=-1, keepdims=True))
                alpha = jnp.exp(m_old - m_new)
                p = jnp.exp(s - m_new)
                l_new = alpha * l_old + jnp.sum(p, axis=-1, keepdims=True)
                p = p.astype(_BF)
                pv = _dot(p[:, :PC], pieces[0][...])
                for j in range(1, G):
                    pv = pv + _dot(p[:, j * PC:(j + 1) * PC], pieces[j][...])
                acc = alpha * acc + pv
                return m_new, l_new, acc

            state0 = (jnp.full((H, 1), -jnp.inf, _F32), jnp.zeros((H, 1), _F32),
                      jnp.zeros((H, Dc), _F32))
            _, l, acc = lax.fori_loop(0, G, slot_c, state0)
            ctx = acc / l
            for k in range(nck):
                cabs_s[k, pl.ds(b, H, stride=B), :] = ctx[:, k * 128:(k + 1) * 128]

            def slot_kv(j, carry2):
                wait_kv(b, j)

                @pl.when(b < B - 1)
                def _():
                    start_spread(c_hbm, c_s, b + 1, j)

                @pl.when(b == B - 1)
                def _():
                    start_spread(wuv_hbm, wuv_s, 0, j)

                rows8 = pl.ds(b + j * 8 * B, 8, stride=B)
                q8 = qb_s[rows8, :].astype(_BF)
                r0 = pl.ds(pl.multiple_of((b * Hkv + 2 * j) * W, W), W)
                r1 = pl.ds(pl.multiple_of((b * Hkv + 2 * j + 1) * W, W), W)
                sb = jnp.where(first, _dot_nt(q8, k_s[r0, :]), _dot_nt(q8, k_s[r1, :]))
                mb = jnp.max(sb, axis=-1, keepdims=True)
                pb = jnp.exp(sb - mb)
                lb = jnp.sum(pb, axis=-1, keepdims=True)
                pb = pb.astype(_BF)
                ob = jnp.where(first, _dot(pb, v_s[r0, :]), _dot(pb, v_s[r1, :]))
                ob_s[rows8, :] = ob / lb
                return carry2

            lax.fori_loop(0, G, slot_kv, 0)
            return carry

        lax.fori_loop(0, B, batch_body, 0)
        obl_s[...] = jnp.concatenate(
            [ob_s[h * B:(h + 1) * B, :] for h in range(Hq)], axis=1).astype(_BF)

        def slot_wuv(g, carry):
            wait_spread(wuv_hbm, wuv_s, 0, g)
            start_unit(wo_hbm, wo_s, g, g)
            return carry

        lax.fori_loop(0, G, slot_wuv, 0)

        def ctx_fn(h, w):
            rows = pl.ds(pl.multiple_of(h * B, B), B)
            lhs = jnp.concatenate([cabs_s[k, rows, :] for k in range(nck)], axis=1)
            ctx_s[rows, :] = _dot(lhs.astype(_BF), w)

        def slot_wo(g, acc):
            wait_unit(wo_hbm, wo_s, g, g)

            @pl.when(g < G - 1)
            def _():
                start_rows(bwo_hbm, bwo_s, g * (8 * Dh), 8 * Dh, g, 4)

            @pl.when(g == G - 1)
            def _():
                start_rows(bwo_hbm, bwo_s, 24 * Dh, 4 * Dh, G - 1, 4)

            _for_head_group(wuv_s, Dc, H, g, ctx_fn)
            lhs = jnp.concatenate(
                [ctx_s[pl.ds(pl.multiple_of((g * 8 + r) * B, B), B), :] for r in range(8)],
                axis=1).astype(_BF)
            rows = pl.ds(pl.multiple_of(g * (8 * D), 8 * D), 8 * D)
            return acc + _dot(lhs, wo_s[rows, :])

        out_a = lax.fori_loop(0, G, slot_wo, jnp.zeros((B, M), _F32))

        def slot_bwo(g, acc):
            row0 = pl.multiple_of(g * (8 * Dh), 8 * Dh)
            wait_rows(bwo_hbm, bwo_s, row0, 8 * Dh, g)

            @pl.when(g < 2)
            def _():
                start_rows(bwo_hbm, bwo_s, (28 + 2 * g) * Dh, 2 * Dh, g, 2)

            rows = pl.ds(row0, 8 * Dh)
            return acc + _dot(obl_s[:, rows], bwo_s[rows, :])

        out_b = lax.fori_loop(0, 3, slot_bwo, jnp.zeros((B, M), _F32))
        for lo, hi, s in ((24, 28, 3), (28, 30, 0), (30, 32, 1)):
            wait_rows(bwo_hbm, bwo_s, lo * Dh, (hi - lo) * Dh, s)
            out_b = out_b + _dot(obl_s[:, lo * Dh:hi * Dh], bwo_s[lo * Dh:hi * Dh, :])

        out = gate * out_a + (1.0 - gate) * out_b
        o_ref[...] = out.astype(o_ref.dtype)

    any_spec = pl.BlockSpec(memory_space=pl.ANY)
    scratch = [
        pltpu.VMEM((B, M), _BF),
        pltpu.VMEM((M,), _BF),
        pltpu.VMEM((B * Sk, Dc), _BF),
        pltpu.VMEM((M * H, D), _BF),
        pltpu.VMEM((Dc * H, D), _BF),
        pltpu.VMEM((Dc * H, D), _BF),
        pltpu.VMEM((H * D, M), _BF),
        pltpu.VMEM((B * Hkv * W, Dh), _BF),
        pltpu.VMEM((B * Hkv * W, Dh), _BF),
        pltpu.VMEM((M, Hq * Dh), _BF),
        pltpu.VMEM((Hq * Dh, M), _BF),
        pltpu.VMEM((Hq * B, Dh), _F32),
        pltpu.VMEM((H * B, D), _F32),
        pltpu.VMEM((nck, H * B, 128), _F32),
        pltpu.VMEM((nck, H * B, 128), _F32),
        pltpu.VMEM((H * B, D), _F32),
        pltpu.VMEM((Hq * B, Dh), _F32),
        pltpu.VMEM((B, Hq * Dh), _BF),
        pltpu.SemaphoreType.DMA((G,)),
    ]
    out = pl.pallas_call(
        kernel,
        out_shape=jax.ShapeDtypeStruct((B, M), A_x.dtype),
        in_specs=[any_spec] * 11,
        out_specs=pl.BlockSpec(memory_space=pltpu.VMEM),
        scratch_shapes=scratch,
        compiler_params=pltpu.CompilerParams(vmem_limit_bytes=110 * 2**20),
    )(A_x.reshape(B, M), A_c_kv.reshape(B * Sk, Dc), A_w_q.reshape(M * H, D),
      A_w_uk.reshape(Dc * H, D), A_w_uv.reshape(Dc * H, D), A_w_o.reshape(H * D, M),
      B_k_cache.reshape(B * Hkv * SkB, Dh), B_v_cache.reshape(B * Hkv * SkB, Dh),
      B_wq, B_wo, gate_w)
    return out.reshape(B, Sq, M)
```
